```python
import jax
import jax.numpy as jnp

def _softmax(x, axis=-1):
    return jax.nn.softmax(x, axis=axis)
def _gelu(x):
    return jax.nn.gelu(x, approximate=True)
def _silu(x):
    return jax.nn.silu(x)
def _sigmoid(x):
    return jax.nn.sigmoid(x)
def _layernorm(x, axis=-1, eps=1e-5):
    m = jnp.mean(x, axis=axis, keepdims=True)
    v = jnp.var(x, axis=axis, keepdims=True)
    return (x - m) / jnp.sqrt(v + eps)
def _scatter_add(tgt, idx, src, axis=0):
    return tgt.at[idx].add(src)
def _segment_sum(src, seg, n):
    return jax.ops.segment_sum(src, seg, n)
class _Rng:
    def __init__(self, key):
        self._k = key
    def _next(self):
        self._k, sub = jax.random.split(self._k)
        return sub
    def normal(self, shape):
        return jax.random.normal(self._next(), shape, dtype=jnp.bfloat16)
    def randint(self, lo, hi, shape):
        return jax.random.randint(self._next(), shape, lo, hi, dtype=jnp.int32)
    def uniform(self, shape, lo=0.0, hi=1.0):
        return jax.random.uniform(self._next(), shape, jnp.bfloat16, lo, hi)
    def permutation(self, n):
        return jax.random.permutation(self._next(), n)


kernel_name = 'recurrent_scan__mha_block_cached__moe_arch_mod__prompt'

def setup_inputs():
    _rng = _Rng(jax.random.key(int.from_bytes(__import__("os").urandom(4), "little")))
    _w = (lambda a: (lambda t: t.astype(jnp.bfloat16) if jnp.issubdtype(t.dtype, jnp.floating) else t)(jnp.asarray(a)))
    def _A_setup():
        B, Sq, D = 1, 2048, 640
        H, Sk, Dh = 32, 2048, 128
        return {
            "x": _w((lambda *s: _rng.normal(s) * 0.05)(B, Sq, D)),
            "k_cache": _w((lambda *s: _rng.normal(s) * 0.05)(B, H, Sk, Dh)),
            "v_cache": _w((lambda *s: _rng.normal(s) * 0.05)(B, H, Sk, Dh)),
            "wq": _w((lambda *s: _rng.normal(s) * 0.05)(D, H * Dh) * (D ** -0.5)),
            "wo": _w((lambda *s: _rng.normal(s) * 0.05)(H * Dh, D) * ((H * Dh) ** -0.5)),
        }
    _A_in = _A_setup()

    def _B_setup():
        B, S, D, F, C = 1, 2048, 640, 1728, 8
        return {
            "x": _w((lambda *s: _rng.normal(s) * 0.05)(B, S, D)),
            "w_r": _w((lambda *s: _rng.normal(s) * 0.05)(D)),
            "w_gate": _w((lambda *s: _rng.normal(s) * 0.05)(D, F)),
            "w_up": _w((lambda *s: _rng.normal(s) * 0.05)(D, F)),
            "w_down": _w((lambda *s: _rng.normal(s) * 0.05)(F, D)),
        }
    _B_in = _B_setup()

    return {
        "A_x": _A_in["x"],
        "A_k_cache": _A_in["k_cache"],
        "A_v_cache": _A_in["v_cache"],
        "A_wq": _A_in["wq"],
        "A_wo": _A_in["wo"],
        "B_x": _B_in["x"],
        "B_w_r": _B_in["w_r"],
        "B_w_gate": _B_in["w_gate"],
        "B_w_up": _B_in["w_up"],
        "B_w_down": _B_in["w_down"],
    }

def reference(A_x, A_k_cache, A_v_cache, A_wq, A_wo, B_x, B_w_r, B_w_gate, B_w_up, B_w_down):
    def _A_ref(x, k_cache, v_cache, wq, wo):
        B, Sq, D = x.shape
        H, Dh = 32, 128
        q = (lambda x, *d: x.transpose(*d))((x @ wq).reshape(B, Sq, H, Dh), 0, 2, 1, 3)
        scores = jnp.einsum("bhqd,bhkd->bhqk", q, k_cache) * (Dh ** -0.5)
        p = _softmax(scores, axis=-1)
        o = jnp.einsum("bhqk,bhkd->bhqd", p, v_cache)
        return (lambda x, *d: x.transpose(*d))(o, 0, 2, 1, 3).reshape(B, Sq, H * Dh) @ wo

    def _B_ref(x, w_r, w_gate, w_up, w_down):
        B, S, D = x.shape
        C = 8
        r = x @ w_r
        idx = jnp.argsort(-r, axis=-1)[:, :C]
        idx_e = jnp.repeat(idx.reshape(B, C, 1), D, axis=2)
        x_sel = jnp.take_along_axis(x, idx_e, axis=1)
        g = _silu(x_sel @ w_gate)
        u = x_sel @ w_up
        y = (g * u) @ w_down
        r_sel = _sigmoid(jnp.take_along_axis(r, idx, axis=1))
        y = y * r_sel.reshape(B, C, 1)
        b_off = (jnp.arange(B) * S).reshape(B, 1)
        flat_idx = (idx + b_off).reshape(B * C)
        zero = (x * 0.0).reshape(B * S, D)
        upd = _scatter_add(zero, flat_idx, y.reshape(B * C, D), axis=0)
        return x + upd.reshape(B, S, D)

    x = A_x
    xn = _layernorm(x, axis=-1)
    s = _A_ref(xn, A_k_cache, A_v_cache, A_wq, A_wo)
    g = _silu(_B_ref(xn, B_w_r, B_w_gate, B_w_up, B_w_down))
    return x + s * g
```

```python
import functools
import jax, jax.numpy as jnp, numpy as np
from jax import lax
from jax.experimental import pallas as pl
from jax.experimental.pallas import tpu as pltpu

S, D, H, DH, F, C = 2048, 640, 32, 128, 1728, 8
f32, bf16 = jnp.float32, jnp.bfloat16

def _build(TQ=1024):
    def kernel(x_ref, k_ref, v_ref, wq_ref, wo_ref, wr_ref, wg_ref, wu_ref, wd_ref, out_ref, xn_ref, acc_ref):
        h = pl.program_id(0)

        @pl.when(h == 0)
        def _():
            def body(i, c):
                r = pl.ds(pl.multiple_of(i * 256, 256), 256)
                x = x_ref[r, :].astype(f32)
                m = jnp.mean(x, axis=-1, keepdims=True)
                xc = x - m
                v = jnp.mean(xc * xc, axis=-1, keepdims=True)
                xn_ref[r, :] = (xc * lax.rsqrt(v + 1e-5)).astype(bf16)
                acc_ref[r, :] = jnp.zeros((256, D), f32)
                return c
            lax.fori_loop(0, S // 256, body, 0)

        def tile(i, c):
            r = pl.ds(pl.multiple_of(i * TQ, TQ), TQ)
            q = jnp.dot(xn_ref[r, :], wq_ref[...], preferred_element_type=f32)
            q = (q * (DH ** -0.5 * 1.4426950408889634)).astype(bf16)
            s = lax.dot_general(q, k_ref[...], (((1,), (1,)), ((), ())), preferred_element_type=f32)
            m = jnp.max(s, axis=-1, keepdims=True)
            p = jnp.exp2(s - m)
            l = jnp.sum(p, axis=-1, keepdims=True)
            o = jnp.dot(p.astype(bf16), v_ref[...], preferred_element_type=f32)
            o = (o / l).astype(bf16)
            acc_ref[r, :] += jnp.dot(o, wo_ref[...], preferred_element_type=f32)
            return c
        lax.fori_loop(0, S // TQ, tile, 0)

        @pl.when(h == H - 1)
        def _():
            r = lax.dot_general(jnp.broadcast_to(wr_ref[...], (8, D)), xn_ref[...], (((1,), (1,)), ((), ())),
                                preferred_element_type=f32)
            r = r.astype(bf16).astype(f32)
            lane = lax.broadcasted_iota(jnp.int32, (8, S), 1)
            row = lax.broadcasted_iota(jnp.int32, (8, S), 0)
            work = r
            onehot = jnp.zeros((8, S), f32)
            for c in range(C):
                mx = jnp.max(work, axis=-1, keepdims=True)
                idx = jnp.min(jnp.where(work == mx, lane, S), axis=-1, keepdims=True)
                hit = lane == idx
                onehot = jnp.where(hit & (row == c), 1.0, onehot)
                work = jnp.where(hit, -jnp.inf, work)
            rsel = jnp.sum(jnp.where(onehot > 0, r, 0.0), axis=-1, keepdims=True)
            xsel = jnp.dot(onehot.astype(bf16), xn_ref[...], preferred_element_type=f32).astype(bf16)
            g = jnp.dot(xsel, wg_ref[...], preferred_element_type=f32)
            u = jnp.dot(xsel, wu_ref[...], preferred_element_type=f32)
            hh = (g * jax.nn.sigmoid(g) * u).astype(bf16)
            y = jnp.dot(hh, wd_ref[...], preferred_element_type=f32) * jax.nn.sigmoid(rsel)
            yb = y.astype(bf16)
            def body(i, c):
                rr = pl.ds(pl.multiple_of(i * 256, 256), 256)
                li = lax.broadcasted_iota(jnp.int32, (8, 256), 1) + i * 256
                return c
            oh = onehot.astype(bf16)
            for i in range(S // 256):
                rr = pl.ds(i * 256, 256)
                upd = lax.dot_general(oh[:, i * 256:(i + 1) * 256], yb, (((0,), (0,)), ((), ())), preferred_element_type=f32)
                b = xn_ref[rr, :].astype(f32) + upd
                gate = b * jax.nn.sigmoid(b)
                out_ref[rr, :] = (x_ref[rr, :].astype(f32) + acc_ref[rr, :] * gate).astype(bf16)

    def fn(A_x, A_k_cache, A_v_cache, A_wq, A_wo, B_x, B_w_r, B_w_gate, B_w_up, B_w_down):
        whole = lambda shape: pl.BlockSpec(shape, lambda h: (0,) * len(shape), pipeline_mode=pl.Buffered(1))
        out = pl.pallas_call(
            kernel,
            grid=(H,),
            in_specs=[
                whole((S, D)),
                pl.BlockSpec((None, S, DH), lambda h: (h, 0, 0)),
                pl.BlockSpec((None, S, DH), lambda h: (h, 0, 0)),
                pl.BlockSpec((D, DH), lambda h: (0, h)),
                pl.BlockSpec((DH, D), lambda h: (h, 0)),
                whole((1, D)), whole((D, F)), whole((D, F)), whole((F, D)),
            ],
            out_specs=pl.BlockSpec((S, D), lambda h: (0, 0)),
            out_shape=jax.ShapeDtypeStruct((S, D), bf16),
            scratch_shapes=[pltpu.VMEM((S, D), bf16), pltpu.VMEM((S, D), f32)],
            compiler_params=pltpu.CompilerParams(dimension_semantics=("arbitrary",), vmem_limit_bytes=100 * 2**20),
        )(A_x.reshape(S, D), A_k_cache.reshape(H, S, DH), A_v_cache.reshape(H, S, DH), A_wq, A_wo,
          B_w_r.reshape(1, D), B_w_gate, B_w_up, B_w_down)
        return out.reshape(1, S, D)
    return fn


_fn = _build()


@jax.jit
def pallas_recurrent_scan__mha_block_cached__moe_arch_mod__prompt_kernel(
    A_x, A_k_cache, A_v_cache, A_wq, A_wo, B_x, B_w_r, B_w_gate, B_w_up, B_w_down
):
    return _fn(A_x, A_k_cache, A_v_cache, A_wq, A_wo, B_x, B_w_r, B_w_gate, B_w_up, B_w_down)
```

```python
import jax, jax.numpy as jnp, numpy as np
from jax import lax
from jax.experimental import pallas as pl
from jax.experimental.pallas import tpu as pltpu

S, D, H, DH, F, C = 2048, 640, 32, 128, 1728, 8
f32, bf16, i32 = jnp.float32, jnp.bfloat16, jnp.int32
NT = (((1,), (1,)), ((), ()))
QSCALE = float(DH ** -0.5 * np.log2(np.e))
EPS_BF16 = float(np.float32(1.00135803e-05))


def _fold(xs, op):
    r = xs[0]
    for a in xs[1:]:
        r = op(r, a)
    return r


def _cols(a):
    return [a[:, j * 128:(j + 1) * 128] for j in range(a.shape[1] // 128)]


def _rb(a):
    return a.astype(bf16).astype(f32)


def _sigmoid(a):
    return 1.0 / (1.0 + jnp.exp(-a))


def _build(T0=256, T1=256, TQ=256, HB=1, T3=512, S3=256, CK=512, flags=None, nobc=False):
    NB = 8
    FB = 256
    NX = S // T0
    NC = S // CK
    NJ = CK // 128

    def kernel(x_hbm, k_hbm, v_hbm, wq_hbm, wo_hbm, wr_ref, wg_hbm, wu_hbm, wd_hbm, out_hbm,
               x_vm, xn_vm, gate_vm, q_vm, o_vm, wq_vm, wo_vm, wg_vm, wu_vm, wd_vm, k_vm, v_vm, out_vm,
               key_vm, sel_vm, y_vm, x_sem, wq_sem, wf_sem, wo_sem, kv_sem, out_sem):

        def x_copy(i):
            r = pl.ds(i * T0, T0)
            return pltpu.make_async_copy(x_hbm.at[r, :], x_vm.at[r, :], x_sem.at[i])

        def wq_copy(j):
            return pltpu.make_async_copy(wq_hbm.at[:, pl.ds(pl.multiple_of(j * 512, 512), 512)], wq_vm.at[j], wq_sem.at[j])

        def wf_copies():
            return [pltpu.make_async_copy(wg_hbm, wg_vm, wf_sem.at[0]),
                    pltpu.make_async_copy(wu_hbm, wu_vm, wf_sem.at[1]),
                    pltpu.make_async_copy(wd_hbm, wd_vm, wf_sem.at[2])]

        def wo_copy():
            return pltpu.make_async_copy(wo_hbm, wo_vm, wo_sem.at[0])

        def kv_copies(g, slot):
            hs = pl.ds(g * HB, HB)
            return [pltpu.make_async_copy(k_hbm.at[hs], k_vm.at[slot], kv_sem.at[0, slot]),
                    pltpu.make_async_copy(v_hbm.at[hs], v_vm.at[slot], kv_sem.at[1, slot])]

        x_copy(0).start()
        wq_copy(0).start()
        for i in range(1, NX):
            x_copy(i).start()
        wq_copy(1).start()
        for cp in wf_copies():
            cp.start()

        wr = wr_ref[...].astype(f32)
        lane = lax.broadcasted_iota(i32, (8, 128), 1)
        sub = lax.broadcasted_iota(i32, (8, 128), 0)

        def layernorm(i, rpack):
            r = pl.ds(i * T0, T0)
            x = x_vm[r, :].astype(f32)
            mean = jnp.sum(x, axis=-1, keepdims=True) * (1.0 / D)
            xc = x - mean
            var = jnp.sum(xc * xc, axis=-1, keepdims=True) * (1.0 / D)
            den = _rb(jnp.sqrt(_rb(_rb(var) + EPS_BF16)))
            xnb = (_rb(x - _rb(mean)) * (1.0 / den)).astype(bf16)
            xn_vm[r, :] = xnb
            xn = xnb.astype(f32)
            gate_vm[r, :] = xn * _sigmoid(xn)
            score = jnp.broadcast_to(jnp.sum(xn * wr, axis=-1, keepdims=True), (T0, 128))
            for g in range(T0 // 8):
                n = i * (T0 // 8) + g
                rpack[n // 128] = jnp.where(lane == n % 128, score[g * 8:(g + 1) * 8, :], rpack[n // 128])
            return xnb

        def qproj(j, r, xnb):
            q = jnp.dot(xnb, wq_vm[j], preferred_element_type=f32) * QSCALE
            for c, qc in enumerate(_cols(q)):
                q_vm[j * 4 + c, r, :] = qc.astype(bf16)

        rpack = [jnp.zeros((8, 128), f32), jnp.zeros((8, 128), f32)]
        for i in range(NX):
            x_copy(i).wait()
            xnb = layernorm(i, rpack)
            if i == 0:
                wq_copy(0).wait()
            qproj(0, pl.ds(i * T0, T0), xnb)
        for a in range(2):
            rb = _rb(rpack[a])
            rb = jnp.where(rb == 0.0, 0.0, rb)
            bits = lax.shift_right_logical(pltpu.bitcast(rb, i32), 16)
            u = jnp.where(bits >= 0x8000, 0xFFFF - bits, bits + 0x8000)
            u = jnp.where(rb != rb, 0, u)
            idx = a * 1024 + lane * 8 + sub
            key_vm[a] = pltpu.bitcast((1 << 29) + u * 2048 + (S - 1 - idx), f32)
        y_vm[...] = jnp.zeros_like(y_vm)

        for j in range(2, NB):
            wq_copy(j).start()
        for cp in kv_copies(0, 0):
            cp.start()
        wo_copy().start()
        for cp in wf_copies():
            cp.wait()

        def top_tokens():
            k0, k1 = key_vm[0], key_vm[1]
            keys = jnp.zeros((8, 128), f32)
            xsel = jnp.zeros((8, D), f32)
            row16 = lax.broadcasted_iota(i32, (16, D), 0)
            row8 = lax.broadcasted_iota(i32, (8, D), 0)
            for c in range(C):
                mx = jnp.max(jnp.max(jnp.maximum(k0, k1), axis=1, keepdims=True), axis=0, keepdims=True)
                k0 = jnp.where(k0 == mx, 0.0, k0)
                k1 = jnp.where(k1 == mx, 0.0, k1)
                keys = jnp.where(sub == c, mx, keys)
                tok = (S - 1) - (pltpu.bitcast(jnp.broadcast_to(mx, (8, 128)), i32)[0, 0] & (S - 1))
                grp = xn_vm[pl.ds(pl.multiple_of((tok >> 4) << 4, 16), 16), :].astype(f32)
                rowv = jnp.sum(jnp.where(row16 == (tok & 15), grp, 0.0), axis=0, keepdims=True)
                xsel = jnp.where(row8 == c, rowv, xsel)
            return keys, xsel

        def phase1(j, carry):
            wq_copy(j).wait()
            keys, xsel = top_tokens()
            sel_vm[:, 0:D] = xsel
            sel_vm[:, D:D + 128] = keys
            xs = jnp.concatenate([xsel, xsel], axis=0).astype(bf16)
            first = (j - 1) * FB
            f0 = pl.multiple_of(jnp.minimum(first, F - FB), 64)
            n1 = S // T1
            gu = None
            for i in range(n1):
                r = pl.ds(i * T1, T1)
                qproj(j, r, xn_vm[r, :])
                if i == n1 // 2:
                    w = jnp.concatenate([wg_vm[pl.ds(f0, FB), :], wu_vm[pl.ds(f0, FB), :]], axis=0)
                    gu = lax.dot_general(xs, w, NT, preferred_element_type=f32)
                    g, u = gu[:, :FB], gu[:, FB:]
                    col = f0 + lax.broadcasted_iota(i32, (16, FB), 1)
                    hid = jnp.where(col >= first, g * _sigmoid(g) * u, 0.0).astype(bf16)
                if i == n1 // 2 + 1:
                    y_vm[...] += jnp.dot(hid, wd_vm[pl.ds(f0, FB), :], preferred_element_type=f32)
            return carry

        lax.fori_loop(1, NB, phase1, 0)

        NG = H // HB

        def phase2(g, carry):
            slot = g & 1
            for cp in kv_copies(g, slot):
                cp.wait()
            for cp in kv_copies(jnp.minimum(g + 1, NG - 1), 1 - slot):
                cp.start()
            zero = lax.shift_right_logical(g, 8)

            def after(m, *ds):
                ds = [pltpu.bitcast(d, i32) for d in ds if d is not None]
                if not ds:
                    return m
                return pltpu.bitcast(pltpu.bitcast(m, i32) | (_fold(ds, jnp.bitwise_or) & zero), f32)

            class Tile:
                pass

            def qk(n):
                st = Tile()
                st.hh, st.r = n // (S // TQ), pl.ds((n % (S // TQ)) * TQ, TQ)
                st.s, st.mps, st.lp = [], [], None
                q = q_vm[g * HB + st.hh, st.r, :]
                for c in range(NC):
                    s = _cols(lax.dot_general(q, k_vm[slot, st.hh, c * CK:(c + 1) * CK, :], NT, preferred_element_type=f32))
                    mc = _fold(s, jnp.maximum)
                    st.mps.append(mc if c == 0 else jnp.maximum(st.mps[-1], mc))
                    st.s.append(s)
                st.m = jnp.broadcast_to(jnp.max(st.mps[-1], axis=-1, keepdims=True), (TQ, 128))
                return st

            def probs(st, c, deps):
                if len(deps) == 1:
                    mm = after(st.m, deps[0], st.lp)
                    ps = [jnp.exp2(s - mm) for s in st.s[c]]
                    lc = _fold(ps, jnp.add)
                    st.lp = lc if st.lp is None else st.lp + lc
                else:
                    ps = []
                    for s, d in zip(st.s[c], deps):
                        p = jnp.exp2(s - after(st.m, d, st.lp))
                        st.lp = p if st.lp is None else st.lp + p
                        ps.append(p)
                return jnp.concatenate(ps, axis=1).astype(bf16)

            NU = HB * (S // TQ)
            cur = qk(0)
            last = None
            for n in range(NU):
                nxt = qk(n + 1) if n + 1 < NU else None
                for c in range(NC):
                    if n == 0 and c == 0:
                        p = probs(cur, 0, [nxt.mps[j * NC // NJ] for j in range(NJ)])
                    else:
                        p = probs(cur, c, [last])
                    oc = jnp.dot(p, v_vm[slot, cur.hh, c * CK:(c + 1) * CK, :], preferred_element_type=f32)
                    last = oc if c == 0 else last + oc
                l = jnp.sum(cur.lp, axis=-1, keepdims=True)
                rl = pl.reciprocal(l, approx=True)
                rl = rl * (2.0 - l * rl)
                last = last * rl
                o_vm[g * HB + cur.hh, cur.r, :] = last.astype(bf16)
                cur = nxt
            return carry

        lax.fori_loop(0, NG, phase2, 0)
        for cp in kv_copies(NG - 1, NG & 1):
            cp.wait()
        wo_copy().wait()

        def out_copy(n):
            r = pl.ds(pl.multiple_of(n * S3, S3), S3)
            return pltpu.make_async_copy(out_vm.at[r, :], out_hbm.at[r, :], out_sem.at[n])

        def phase3(i, carry):
            xsel = sel_vm[:, 0:D]
            kbits = pltpu.bitcast(sel_vm[:, D:D + 128], i32)
            tok = (S - 1) - (kbits & (S - 1))
            u = lax.shift_right_logical(kbits, 11) & 0xFFFF
            rsel = pltpu.bitcast(jnp.where(u >= 0x8000, u - 0x8000, 0xFFFF - u) << 16, f32)
            b = xsel + y_vm[0:8, :] * jnp.tile(_sigmoid(rsel), (1, D // 128))
            gsel = _cols(b * _sigmoid(b))
            for t in range(T3 // S3):
                n = i * (T3 // S3) + t
                r = pl.ds(pl.multiple_of(n * S3, S3), S3)
                row = n * S3 + lax.broadcasted_iota(i32, (S3, 128), 0)
                hits = [row == tok[c:c + 1, :] for c in range(C)]
                for nn in range(D // 128):
                    cs = slice(nn * 128, (nn + 1) * 128)
                    acc = None
                    for kc in range(H // 4):
                        o = jnp.concatenate([o_vm[kc * 4 + a, r, :] for a in range(4)], axis=1)
                        d = jnp.dot(o, wo_vm[kc * 512:(kc + 1) * 512, cs], preferred_element_type=f32)
                        acc = d if acc is None else acc + d
                    gate = gate_vm[r, cs]
                    for c in range(C):
                        gate = jnp.where(hits[c], gsel[nn][c:c + 1, :], gate)
                    out_vm[r, cs] = (x_vm[r, cs].astype(f32) + acc * gate).astype(bf16)
                out_copy(n).start()
            return carry

        lax.fori_loop(0, S // T3, phase3, 0)
        for n in range(S // S3):
            out_copy(n).wait()

    def fn(A_x, A_k_cache, A_v_cache, A_wq, A_wo, B_x, B_w_r, B_w_gate, B_w_up, B_w_down):
        hbm = pl.BlockSpec(memory_space=pltpu.HBM)
        dma = pltpu.SemaphoreType.DMA
        out = pl.pallas_call(
            kernel,
            in_specs=[hbm, hbm, hbm, hbm, hbm, pl.BlockSpec(memory_space=pltpu.VMEM), hbm, hbm, hbm],
            out_specs=hbm,
            out_shape=jax.ShapeDtypeStruct((S, D), bf16),
            scratch_shapes=[
                pltpu.VMEM((S, D), bf16), pltpu.VMEM((S, D), bf16), pltpu.VMEM((S, D), f32),
                pltpu.VMEM((H, S, DH), bf16), pltpu.VMEM((H, S, DH), bf16),
                pltpu.VMEM((NB, D, 512), bf16), pltpu.VMEM((H * DH, D), bf16),
                pltpu.VMEM((F, D), bf16), pltpu.VMEM((F, D), bf16), pltpu.VMEM((F, D), bf16),
                pltpu.VMEM((2, HB, S, DH), bf16), pltpu.VMEM((2, HB, S, DH), bf16), pltpu.VMEM((S, D), bf16),
                pltpu.VMEM((2, 8, 128), f32), pltpu.VMEM((8, D + 128), f32), pltpu.VMEM((16, D), f32),
                dma((NX,)), dma((NB,)), dma((3,)), dma((1,)), dma((2, 2)), dma((S // S3,)),
            ],
            compiler_params=pltpu.CompilerParams(vmem_limit_bytes=110 * 2**20, flags=flags, disable_bounds_checks=nobc),
        )(A_x.reshape(S, D), A_k_cache.reshape(H, S, DH), A_v_cache.reshape(H, S, DH), A_wq, A_wo,
          B_w_r.reshape(1, D), B_w_gate.T, B_w_up.T, B_w_down)
        return out.reshape(1, S, D)
    return fn


@jax.jit
def pallas_recurrent_scan__mha_block_cached__moe_arch_mod__prompt_kernel(
    A_x, A_k_cache, A_v_cache, A_wq, A_wo, B_x, B_w_r, B_w_gate, B_w_up, B_w_down
):
    return _build()(A_x, A_k_cache, A_v_cache, A_wq, A_wo, B_x, B_w_r, B_w_gate, B_w_up, B_w_down)
```

```python
import contextlib
import jax, jax.numpy as jnp, numpy as np
from jax import lax
from jax.experimental import pallas as pl
from jax.experimental.pallas import tpu as pltpu

S, D, H, DH, F, C = 2048, 640, 32, 128, 1728, 8
f32, bf16, i32 = jnp.float32, jnp.bfloat16, jnp.int32
NT = (((1,), (1,)), ((), ()))
QSCALE = float(DH ** -0.5 * np.log2(np.e))
EPS_BF16 = 1.0013580322265625e-05
KD = D // 128


def _fold(xs, op):
    r = xs[0]
    for a in xs[1:]:
        r = op(r, a)
    return r


def _cols(a, w=128):
    return [a[:, j * w:(j + 1) * w] for j in range(a.shape[1] // w)]


def _rows(a, w):
    return [a[j * w:(j + 1) * w, :] for j in range(a.shape[0] // w)]


def _rb(a):
    return a.astype(bf16).astype(f32)


def _sigmoid(a):
    return 1.0 / (1.0 + jnp.exp(-a))


def _after(val, deps, zero):
    deps = [pltpu.bitcast(d, i32) for d in deps if d is not None]
    if not deps:
        return val
    return pltpu.bitcast(pltpu.bitcast(val, i32) | (_fold(deps, jnp.bitwise_or) & zero), val.dtype)


def _after_rows(lhs, deps, zero):
    if not deps:
        return lhs
    return jnp.concatenate([_after(g, deps.get(n, []), zero) for n, g in enumerate(_rows(lhs, 16))], axis=0)


def _build(XC=(2, 2, 4, 8), T0=128, T1=256, TQ=256, T3=512, S3=256, CK=512, P0=0, NE=0, LEAD=2, kvpos=1, prof=False, flags=None, nobc=False):
    R1 = 512
    FB = 512
    NX = len(XC)
    XO = [sum(XC[:i]) for i in range(NX + 1)]
    assert XO[-1] * T0 == S
    NC = S // CK
    NJ = CK // 128
    scope = jax.named_scope if prof else (lambda name: contextlib.nullcontext())

    def kernel(x_hbm, k_hbm, v_hbm, wq_hbm, wo_hbm, wr_ref, wg_hbm, wu_hbm, wd_hbm, out_hbm,
               x_vm, xn_vm, b_vm, q_vm, o_vm, wq_vm, wo_vm, wf_vm, k_vm, v_vm, out_vm,
               key_vm, sel_vm, y_vm, x_sem, wq_sem, wf_sem, wo_sem, kv_sem, out_sem):

        def x_copy(i):
            r = pl.ds(XO[i] * T0, XC[i] * T0)
            return pltpu.make_async_copy(x_hbm.at[r, :], x_vm.at[r, :], x_sem.at[i])

        def wq_copy(i):
            c = (pl.ds(0, 512), pl.ds(512, 512), pl.ds(1024, 3072))[i]
            return pltpu.make_async_copy(wq_hbm.at[:, c], wq_vm.at[:, c], wq_sem.at[i])

        def f_start(i):
            return min(i * FB, F - FB) if isinstance(i, int) else pl.multiple_of(jnp.minimum(i * FB, F - FB), 64)

        def wf_copies(i):
            r = pl.ds(f_start(i), FB)
            return [pltpu.make_async_copy(w.at[r, :], wf_vm.at[i, a], wf_sem.at[i, a])
                    for a, w in enumerate((wg_hbm, wu_hbm, wd_hbm))]

        def wo_copy():
            return pltpu.make_async_copy(wo_hbm, wo_vm, wo_sem.at[0])

        def kv_copies(h, slot):
            return [pltpu.make_async_copy(k_hbm.at[h], k_vm.at[slot], kv_sem.at[0, slot]),
                    pltpu.make_async_copy(v_hbm.at[h], v_vm.at[slot], kv_sem.at[1, slot])]

        x_copy(0).start()
        wq_copy(0).start()
        wr = wr_ref[...].astype(f32)
        zero0 = lax.shift_right_logical(pltpu.bitcast(jnp.broadcast_to(wr[:, 0:128], (8, 128)), i32) & 1, 1)
        lane = lax.broadcasted_iota(i32, (8, 128), 1)
        sub = lax.broadcasted_iota(i32, (8, 128), 0)
        rpack = [jnp.zeros((8, 128), f32), jnp.zeros((8, 128), f32)]

        def layernorm(r0, n, start=None):
            r = pl.ds(r0, n)
            x = x_vm[r, :]
            if start is not None:
                deps = {g: [d] for g, d in enumerate(_rows(start, 8)[::4][:n // 16])}
                x = jnp.concatenate([_after_rows(xk, deps, zero0) for xk in _cols(x)], axis=1)
            x = x.astype(f32)
            mean = jnp.sum(x, axis=-1, keepdims=True) * (1.0 / D)
            yield mean
            xc = x - mean
            var = jnp.sum(xc * xc, axis=-1, keepdims=True) * (1.0 / D)
            yield var
            inv = 1.0 / _rb(jnp.sqrt(_rb(_rb(var) + EPS_BF16)))
            yield inv
            xnb = (_rb(x - _rb(mean)) * inv).astype(bf16)
            xn_vm[r, :] = xnb
            b_vm[r, :] = xnb
            part = _fold(_cols(xnb.astype(f32) * wr), jnp.add)
            yield part
            score = jnp.broadcast_to(jnp.sum(part, axis=-1, keepdims=True), (n, 128))
            packed = []
            for a, sc in enumerate(_rows(score, 8)):
                g = r0 // 8 + a
                rpack[g // 128] = jnp.where(lane == g % 128, sc, rpack[g // 128])
                packed.append(rpack[g // 128])
            yield jnp.concatenate(packed, axis=0)

        def qproj(r, j, zero, side, barrier=None):
            load = lambda k: (xn_vm[r, k * 128:(k + 1) * 128], wq_vm[k * 128:(k + 1) * 128, j * 512:(j + 1) * 512])
            early = {}
            if barrier is not None:
                early = {k: load(k) for k in range(NE)}
                barrier()
            acc = None
            for k in range(KD):
                deps = side(k, acc)
                lhs, rhs = early[k] if k in early else load(k)
                d = jnp.dot(_after_rows(lhs, deps, zero), rhs, preferred_element_type=f32)
                acc = d if acc is None else acc + d
            for c, qc in enumerate(_cols(acc * QSCALE)):
                q_vm[j * 4 + c, r, :] = qc.astype(bf16)
            return acc

        G0 = T0 // 16
        NT0 = S // T0
        first = XC[0]
        steps = [(t, 0) for t in range(first)] + [(t, 1) for t in range(first)]
        steps += [(t, j) for t in range(first, NT0) for j in range(2)]
        ln_at = {}
        for t in range(first, NT0):
            n = steps.index((t, 0))
            ln_at[n - 3] = t * T0
            ln_at[n - 2] = t * T0 + T0 // 2
        if P0 == 0:
            x_copy(1).start()
        with scope("w_x0"):
            x_copy(0).wait()
        if P0 == 1:
            x_copy(1).start()
        for _ in layernorm(0, first * T0):
            pass
        if P0 == 2:
            x_copy(1).start()
        if P0 <= 2:
            wq_copy(1).start()
        with scope("w_wq0"):
            wq_copy(0).wait()
        if P0 > 2:
            x_copy(1).start()
            wq_copy(1).start()
        running = {}
        for n, (t, j) in enumerate(steps):
            waits = []
            r0 = ln_at.get(n)
            if r0 is not None and r0 % T0 == 0 and r0 // T0 in XO:
                i = XO.index(r0 // T0)
                waits.append(x_copy(i).wait)
                if i == 1:
                    assert j == 0
                    waits.append(wq_copy(1).wait)
                if i + 1 < NX:
                    waits.append(x_copy(i + 1).start)
                else:
                    waits += [wq_copy(2).start] + [cp.start for cp in wf_copies(0)]

            def barrier(waits=waits):
                for a, w in enumerate(waits):
                    with scope(f"w_{n}_{a}"):
                        w()

            def side(k, acc, n=n):
                p = n * KD + k
                if k == 1 and n in ln_at:
                    gen = layernorm(ln_at[n], T0 // 2, acc[:, 0:128])
                    for a in range(5):
                        running[p + LEAD + a] = gen
                if p not in running:
                    return {}
                v = jnp.broadcast_to(next(running.pop(p)), (T0 // 2, 128))
                return {a: [d] for a, d in enumerate(_rows(v, 8))}

            qproj(pl.ds(t * T0, T0), j, zero0, side, barrier if waits else None)
        assert not running
        for a in range(2):
            rb = _rb(rpack[a])
            rb = jnp.where(rb == 0.0, 0.0, rb)
            bits = lax.shift_right_logical(pltpu.bitcast(rb, i32), 16)
            u = jnp.where(bits >= 0x8000, 0xFFFF - bits, bits + 0x8000)
            u = jnp.where(rb != rb, 0, u)
            idx = a * 1024 + lane * 8 + sub
            key_vm[a] = pltpu.bitcast((1 << 29) + u * 2048 + (S - 1 - idx), f32)
        y_vm[...] = jnp.zeros_like(y_vm)
        with scope("w_wq2"):
            wq_copy(2).wait()

        def token_group(tok):
            return pl.ds(pl.multiple_of((tok >> 4) << 4, 16), 16)

        def phase1(i, carry):
            for cp in wf_copies(i):
                cp.wait()
            zero = lax.shift_right_logical(i, 8)
            row16 = lax.broadcasted_iota(i32, (16, D), 0)
            st = dict(k0=key_vm[0], k1=key_vm[1], keys=jnp.zeros((8, 128), f32), xsel=jnp.zeros((16, D), f32),
                      g=None, u=None)

            def pick(c):
                k0, k1 = st["k0"], st["k1"]
                mx = jnp.max(jnp.max(jnp.maximum(k0, k1), axis=1, keepdims=True), axis=0, keepdims=True)
                st["k0"] = jnp.where(k0 == mx, 0.0, k0)
                st["k1"] = jnp.where(k1 == mx, 0.0, k1)
                st["keys"] = jnp.where(sub == c, mx, st["keys"])
                tok = (S - 1) - (pltpu.bitcast(jnp.broadcast_to(mx, (8, 128)), i32)[0, 0] & (S - 1))
                grp = xn_vm[token_group(tok), :].astype(f32)
                rowv = jnp.sum(jnp.where(row16 == (tok & 15), grp, 0.0), axis=0, keepdims=True)
                st["xsel"] = jnp.where(row16 == c, rowv, st["xsel"])
                return {0: [st["keys"]]}

            def gathered():
                sel_vm[:, 0:D] = st["xsel"][0:8, :]
                sel_vm[:, D:D + 128] = st["keys"]
                st["xs"] = st["xsel"].astype(bf16)
                return {0: _cols(st["xs"])}

            def gate_up(a, k):
                d = lax.dot_general(st["xs"][:, k * 128:(k + 1) * 128], wf_vm[i, a, :, k * 128:(k + 1) * 128], NT,
                                    preferred_element_type=f32)
                name = "gu"[a]
                st[name] = d if k == 0 else st[name] + d
                return {}

            def hidden():
                col = f_start(i) + lax.broadcasted_iota(i32, (16, FB), 1)
                g = st["g"]
                st["hid"] = jnp.where(col >= i * FB, g * _sigmoid(g) * st["u"], 0.0).astype(bf16)
                return {0: _cols(st["hid"])}

            def down(n):
                cs = slice(n * 128, (n + 1) * 128)
                y_vm[:, cs] += jnp.dot(st["hid"], wf_vm[i, 2, :, cs], preferred_element_type=f32)
                return {}

            def prefetch():
                @pl.when(i + 1 < S // R1)
                def _():
                    for cp in wf_copies(i + 1):
                        cp.start()

                @pl.when(i + 1 == S // R1)
                def _():
                    for cp in kv_copies(0, 0):
                        cp.start()
                    wo_copy().start()

            prefetch()
            tasks = {2 * c + 2: (lambda c=c: pick(c)) for c in range(C)}
            tasks[20] = gathered
            for a in range(2):
                for k in range(KD):
                    tasks[22 + a * KD + k] = lambda a=a, k=k: gate_up(a, k)
            tasks[35] = hidden
            for n in range(KD):
                tasks[37 + n] = lambda n=n: down(n)
            cnt = 0
            for t in range(R1 // T1):
                r = pl.ds(pl.multiple_of(i * R1 + t * T1, T1), T1)
                for j in range(2, 8):
                    qproj(r, j, zero, lambda k, acc, cnt=cnt: tasks[cnt + k]() if cnt + k in tasks else {})
                    cnt += KD
            assert cnt > max(tasks)
            return carry

        with scope("p1"):
            lax.fori_loop(0, S // R1, phase1, 0)

        kbits = pltpu.bitcast(sel_vm[:, D:D + 128], i32)
        u = lax.shift_right_logical(kbits, 11) & 0xFFFF
        rsel = pltpu.bitcast(jnp.where(u >= 0x8000, u - 0x8000, 0xFFFF - u) << 16, f32)
        bsel = sel_vm[:, 0:D] + y_vm[0:8, :] * jnp.tile(_sigmoid(rsel), (1, KD))
        row16 = lax.broadcasted_iota(i32, (16, D), 0)
        for c in range(C):
            tok = (S - 1) - (kbits[c, 0] & (S - 1))
            grp = b_vm[token_group(tok), :].astype(f32)
            b_vm[token_group(tok), :] = jnp.where(row16 == (tok & 15), bsel[c:c + 1, :], grp).astype(bf16)

        def phase2(h, carry):
            slot = h & 1
            for cp in kv_copies(h, slot):
                cp.wait()

            def prefetch():
                for cp in kv_copies(jnp.minimum(h + 1, H - 1), 1 - slot):
                    cp.start()

            zero = lax.shift_right_logical(h, 8)

            class Tile:
                pass

            def qk(n):
                st = Tile()
                st.r = pl.ds(n * TQ, TQ)
                st.s, st.mps, st.lp = [], [], None
                q = q_vm[h, st.r, :]
                for c in range(NC):
                    s = _cols(lax.dot_general(q, k_vm[slot, c * CK:(c + 1) * CK, :], NT, preferred_element_type=f32))
                    mc = _fold(s, jnp.maximum)
                    st.mps.append(mc if c == 0 else jnp.maximum(st.mps[-1], mc))
                    st.s.append(s)
                st.m = jnp.broadcast_to(jnp.max(st.mps[-1], axis=-1, keepdims=True), (TQ, 128))
                return st

            def probs(st, c, deps):
                if len(deps) == 1:
                    mm = _after(st.m, [deps[0], st.lp], zero)
                    ps = [jnp.exp2(s - mm) for s in st.s[c]]
                    lc = _fold(ps, jnp.add)
                    st.lp = lc if st.lp is None else st.lp + lc
                else:
                    ps = []
                    for s, d in zip(st.s[c], deps):
                        p = jnp.exp2(s - _after(st.m, [d, st.lp], zero))
                        st.lp = p if st.lp is None else st.lp + p
                        ps.append(p)
                return jnp.concatenate(ps, axis=1).astype(bf16)

            NU = S // TQ
            if kvpos == 0:
                prefetch()
            cur = qk(0)
            if kvpos == 1:
                prefetch()
            last = None
            for n in range(NU):
                nxt = qk(n + 1) if n + 1 < NU else None
                for c in range(NC):
                    if n == 0 and c == 0:
                        p = probs(cur, 0, [nxt.mps[j * NC // NJ] for j in range(NJ)])
                    else:
                        p = probs(cur, c, [last])
                    oc = jnp.dot(p, v_vm[slot, c * CK:(c + 1) * CK, :], preferred_element_type=f32)
                    last = oc if c == 0 else last + oc
                l = jnp.sum(cur.lp, axis=-1, keepdims=True)
                rl = pl.reciprocal(l, approx=True)
                rl = rl * (2.0 - l * rl)
                last = last * rl
                o_vm[h, cur.r, :] = last.astype(bf16)
                cur = nxt
            return carry

        with scope("p2"):
            lax.fori_loop(0, H, phase2, 0)
        for cp in kv_copies(H - 1, H & 1):
            cp.wait()
        wo_copy().wait()

        def out_copy(n):
            r = pl.ds(pl.multiple_of(n * S3, S3), S3)
            return pltpu.make_async_copy(out_vm.at[r, :], out_hbm.at[r, :], out_sem.at[n])

        def phase3(i, carry):
            zero = lax.shift_right_logical(i, 8)
            for t in range(T3 // S3):
                n = i * (T3 // S3) + t
                r = pl.ds(pl.multiple_of(n * S3, S3), S3)
                for nn in range(KD):
                    cs = slice(nn * 128, (nn + 1) * 128)
                    b = b_vm[r, cs].astype(f32)
                    gate = b * _sigmoid(b)
                    gates = _rows(gate, 8)
                    acc = None
                    for kc in range(H // 4):
                        o = [o_vm[kc * 4 + a, r, :] for a in range(4)]
                        if 1 <= kc <= 4:
                            o[0] = _after_rows(o[0], {g: gates[2 * g:2 * g + 2] for g in range(kc - 1, S3 // 16, 4)}, zero)
                        d = jnp.dot(jnp.concatenate(o, axis=1), wo_vm[kc * 512:(kc + 1) * 512, cs], preferred_element_type=f32)
                        acc = d if acc is None else acc + d
                    out_vm[r, cs] = (x_vm[r, cs].astype(f32) + acc * gate).astype(bf16)
                out_copy(n).start()
            return carry

        with scope("p3"):
            lax.fori_loop(0, S // T3, phase3, 0)
        with scope("w_out"):
            for n in range(S // S3):
                out_copy(n).wait()

    def fn(A_x, A_k_cache, A_v_cache, A_wq, A_wo, B_x, B_w_r, B_w_gate, B_w_up, B_w_down):
        hbm = pl.BlockSpec(memory_space=pltpu.HBM)
        dma = pltpu.SemaphoreType.DMA
        out = pl.pallas_call(
            kernel,
            in_specs=[hbm, hbm, hbm, hbm, hbm, pl.BlockSpec(memory_space=pltpu.VMEM), hbm, hbm, hbm],
            out_specs=hbm,
            out_shape=jax.ShapeDtypeStruct((S, D), bf16),
            scratch_shapes=[
                pltpu.VMEM((S, D), bf16), pltpu.VMEM((S, D), bf16), pltpu.VMEM((S, D), bf16),
                pltpu.VMEM((H, S, DH), bf16), pltpu.VMEM((H, S, DH), bf16),
                pltpu.VMEM((D, H * DH), bf16), pltpu.VMEM((H * DH, D), bf16),
                pltpu.VMEM((S // R1, 3, FB, D), bf16),
                pltpu.VMEM((2, S, DH), bf16), pltpu.VMEM((2, S, DH), bf16), pltpu.VMEM((S, D), bf16),
                pltpu.VMEM((2, 8, 128), f32), pltpu.VMEM((8, D + 128), f32), pltpu.VMEM((16, D), f32),
                dma((NX,)), dma((3,)), dma((S // R1, 3)), dma((1,)), dma((2, 2)), dma((S // S3,)),
            ],
            compiler_params=pltpu.CompilerParams(vmem_limit_bytes=110 * 2**20, flags=flags, disable_bounds_checks=nobc),
        )(A_x.reshape(S, D), A_k_cache.reshape(H, S, DH), A_v_cache.reshape(H, S, DH), A_wq, A_wo,
          B_w_r.reshape(1, D), B_w_gate.T, B_w_up.T, B_w_down)
        return out.reshape(1, S, D)
    return fn


@jax.jit
def pallas_recurrent_scan__mha_block_cached__moe_arch_mod__prompt_kernel(
    A_x, A_k_cache, A_v_cache, A_wq, A_wo, B_x, B_w_r, B_w_gate, B_w_up, B_w_down
):
    return _build()(A_x, A_k_cache, A_v_cache, A_wq, A_wo, B_x, B_w_r, B_w_gate, B_w_up, B_w_down)
```

```python
import contextlib
import jax, jax.numpy as jnp, numpy as np
from jax import lax
from jax.experimental import pallas as pl
from jax.experimental.pallas import tpu as pltpu

S, D, H, DH, F, C = 2048, 640, 32, 128, 1728, 8
f32, bf16, i32 = jnp.float32, jnp.bfloat16, jnp.int32
NT = (((1,), (1,)), ((), ()))
QSCALE = float(DH ** -0.5 * np.log2(np.e))
EPS_BF16 = 1.0013580322265625e-05
KD = D // 128


def _fold(xs, op):
    r = xs[0]
    for a in xs[1:]:
        r = op(r, a)
    return r


def _cols(a, w=128):
    return [a[:, j * w:(j + 1) * w] for j in range(a.shape[1] // w)]


def _rows(a, w):
    return [a[j * w:(j + 1) * w, :] for j in range(a.shape[0] // w)]


def _rb(a):
    return a.astype(bf16).astype(f32)


def _sigmoid(a):
    return pl.reciprocal(1.0 + jnp.exp(-a), approx=True)


def _after(val, deps, zero):
    deps = [pltpu.bitcast(d, i32) for d in deps if d is not None]
    if not deps:
        return val
    return pltpu.bitcast(pltpu.bitcast(val, i32) | (_fold(deps, jnp.bitwise_or) & zero), val.dtype)


def _after_rows(lhs, deps, zero):
    if not deps:
        return lhs
    return jnp.concatenate([_after(g, deps.get(n, []), zero) for n, g in enumerate(_rows(lhs, 16))], axis=0)


def _build(XC=(2, 2, 4, 8), T0=128, T1=256, TQ=256, HB=2, DL=(2, 3, 4, 5, 7), T3=256, S3=256, CK=512, P0=0, OC=(2, 4), PK=3, NE=0, LEAD=2, kvpos=1, prof=False, flags=None, nobc=False):
    NB = 8
    FB = 256
    NX = len(XC)
    XO = [sum(XC[:i]) for i in range(NX + 1)]
    assert XO[-1] * T0 == S
    NC = S // CK
    NJ = CK // 128
    scope = jax.named_scope if prof else (lambda name: contextlib.nullcontext())

    def kernel(x_hbm, k_hbm, v_hbm, wq_hbm, wo_hbm, wr_hbm, wg_hbm, wu_hbm, wd_hbm, out_hbm,
               x_vm, xn_vm, b_vm, q_vm, o_vm, wq_vm, wo_vm, wf_vm, kv_vm, out_vm, wr_vm,
               key_vm, sel_vm, y_vm, x_sem, wq_sem, wf_sem, wo_sem, kv_sem, out_sem, wr_sem):

        def x_copy(i):
            r = pl.ds(XO[i] * T0, XC[i] * T0)
            return pltpu.make_async_copy(x_hbm.at[r, :], x_vm.at[r, :], x_sem.at[i])

        def wq_copy(i):
            c = pl.ds(i * 512 if isinstance(i, int) else pl.multiple_of(i * 512, 512), 512)
            return pltpu.make_async_copy(wq_hbm.at[:, c], wq_vm.at[i], wq_sem.at[i & 3])

        def f_start(i):
            return min(i * FB, F - FB) if isinstance(i, int) else pl.multiple_of(jnp.minimum(i * FB, F - FB), 64)

        def wf_copies(i):
            r = pl.ds(f_start(i), FB)
            return [pltpu.make_async_copy(w.at[r, :], wf_vm.at[i, pl.ds(a * FB, FB), :], wf_sem.at[i & 3])
                    for a, w in enumerate((wg_hbm, wu_hbm, wd_hbm))]

        def wo_copy():
            return pltpu.make_async_copy(wo_hbm, wo_vm, wo_sem.at[0])

        def kv_copies(g, slot):
            hs = pl.ds(g * HB, HB)
            return [pltpu.make_async_copy(k_hbm.at[hs], kv_vm.at[slot, 0], kv_sem.at[slot]),
                    pltpu.make_async_copy(v_hbm.at[hs], kv_vm.at[slot, 1], kv_sem.at[slot])]

        def kv_wait(slot):
            pltpu.make_async_copy(kv_vm.at[slot], kv_vm.at[slot], kv_sem.at[slot]).wait()

        x_copy(0).start()
        wq_copy(0).start()
        wr_copy = pltpu.make_async_copy(wr_hbm, wr_vm, wr_sem.at[0])
        wr_copy.start()
        wr_copy.wait()
        wr = wr_vm[...].astype(f32).reshape(1, D)
        zero0 = lax.shift_right_logical(pltpu.bitcast(jnp.broadcast_to(wr[:, 0:128], (8, 128)), i32)[0, 0] & 1, 1)
        lane = lax.broadcasted_iota(i32, (8, 128), 1)
        sub = lax.broadcasted_iota(i32, (8, 128), 0)
        rpack = [jnp.zeros((8, 128), f32), jnp.zeros((8, 128), f32)]

        def layernorm(r0, n, start=None):
            r = pl.ds(r0, n)
            x = x_vm[r, :]
            if start is not None:
                xs = _cols(x.astype(f32))
                x = jnp.concatenate([_after(xs[0], [start], zero0)] + xs[1:], axis=1)
            x = x.astype(f32)
            mean = jnp.sum(x, axis=-1, keepdims=True) * (1.0 / D)
            yield mean
            shift = _rb(mean)
            d = x - shift
            var = jnp.sum(d * d, axis=-1, keepdims=True) * (1.0 / D) - (mean - shift) * (mean - shift)
            yield var
            inv = pl.reciprocal(_rb(jnp.sqrt(_rb(_rb(var) + EPS_BF16))), approx=True)
            yield inv
            xn = d * inv
            xnb = xn.astype(bf16)
            xn_vm[r, :] = xnb
            b_vm[r, :] = xnb
            part = _fold(_cols(xn * wr), jnp.add)
            yield part
            score = jnp.broadcast_to(jnp.sum(part, axis=-1, keepdims=True), (n, 128))
            packed = []
            for a, sc in enumerate(_rows(score, 8)):
                g = r0 // 8 + a
                rpack[g // 128] = jnp.where(lane == g % 128, sc, rpack[g // 128])
                packed.append(rpack[g // 128])
            yield jnp.concatenate(packed, axis=0)

        def qproj(r, j, zero, side, barrier=None):
            load = lambda k: (xn_vm[r, k * 128:(k + 1) * 128], wq_vm[j, k * 128:(k + 1) * 128, :])
            early = {}
            if barrier is not None:
                early = {k: load(k) for k in range(NE)}
                barrier()
            acc = None
            for k in range(KD):
                deps = side(k, acc)
                lhs, rhs = early[k] if k in early else load(k)
                d = jnp.dot(_after_rows(lhs, deps, zero), rhs, preferred_element_type=f32)
                acc = d if acc is None else acc + d
                if k == PK:
                    mark = d[:, 0:128]
            for c, qc in enumerate(_cols(acc * QSCALE)):
                q_vm[j * 4 + c, r, :] = qc.astype(bf16)
            return mark

        NT0 = S // T0
        first = XC[0]
        with scope("w_x0"):
            x_copy(0).wait()
        if P0 == 0:
            x_copy(1).start()
        for _ in layernorm(0, first * T0):
            pass
        if P0 > 0:
            x_copy(1).start()
        with scope("w_wq0"):
            wq_copy(0).wait()
        if P0 < 2:
            x_copy(2).start()
        running = {}
        prev = None
        for n in range(NT0):
            t = n + 1
            waits = []
            if first <= t < NT0 and t in XO:
                i = XO.index(t)
                waits.append(x_copy(i).wait)
                if i + 1 == NX:
                    waits += [wq_copy(1).start] + [cp.start for cp in wf_copies(0)]
                elif i > 1 or P0 >= 2:
                    waits.append(x_copy(i + 1).start)
            for a, w in enumerate(waits):
                with scope(f"w_{n}_{a}"):
                    w()
            if first <= t < NT0:
                gen = layernorm(t * T0, T0, None if waits else prev)
                for a in DL:
                    running.setdefault(n * KD + a, []).append(gen)

            def side(k, acc, n=n):
                vs = [_rows(jnp.broadcast_to(next(gen), (T0, 128)), 8) for gen in running.pop(n * KD + k, [])]
                return {a: [v[2 * a + 1] for v in vs] for a in range(T0 // 16)} if vs else {}

            prev = qproj(pl.ds(n * T0, T0), 0, zero0, side)
        assert not running
        wq_copy(2).start()
        for cp in wf_copies(1):
            cp.start()
        for a in range(2):
            rb = _rb(rpack[a])
            rb = jnp.where(rb == 0.0, 0.0, rb)
            bits = lax.shift_right_logical(pltpu.bitcast(rb, i32), 16)
            u = jnp.where(bits >= 0x8000, 0xFFFF - bits, bits + 0x8000)
            u = jnp.where(rb != rb, 0, u)
            idx = a * 1024 + lane * 8 + sub
            key_vm[a] = pltpu.bitcast((1 << 29) + u * 2048 + (S - 1 - idx), f32)
        y_vm[...] = jnp.zeros_like(y_vm)

        def token_group(tok):
            return pl.ds(pl.multiple_of((tok >> 4) << 4, 16), 16)

        def phase1(i, carry):
            wq_copy(i + 1).wait()
            pltpu.make_async_copy(wf_vm.at[i], wf_vm.at[i], wf_sem.at[i & 3]).wait()
            zero = lax.shift_right_logical(i, 8)
            row16 = lax.broadcasted_iota(i32, (16, D), 0)
            st = dict(k0=key_vm[0], k1=key_vm[1], keys=jnp.zeros((8, 128), f32), xsel=jnp.zeros((16, D), f32),
                      g=None, u=None)

            def pick(c):
                k0, k1 = st["k0"], st["k1"]
                mx = jnp.max(jnp.max(jnp.maximum(k0, k1), axis=1, keepdims=True), axis=0, keepdims=True)
                st["k0"] = jnp.where(k0 == mx, 0.0, k0)
                st["k1"] = jnp.where(k1 == mx, 0.0, k1)
                st["keys"] = jnp.where(sub == c, mx, st["keys"])
                tok = (S - 1) - (pltpu.bitcast(jnp.broadcast_to(mx, (8, 128)), i32)[0, 0] & (S - 1))
                grp = xn_vm[token_group(tok), :].astype(f32)
                rowv = jnp.sum(jnp.where(row16 == (tok & 15), grp, 0.0), axis=0, keepdims=True)
                st["xsel"] = jnp.where(row16 == c, rowv, st["xsel"])
                return {0: [st["keys"]]}

            def gathered():
                sel_vm[:, 0:D] = st["xsel"][0:8, :]
                sel_vm[:, D:D + 128] = st["keys"]
                st["xs"] = st["xsel"].astype(bf16)
                return {0: _cols(st["xs"])}

            def gate_up(k):
                d = lax.dot_general(st["xs"][:, k * 128:(k + 1) * 128], wf_vm[i, 0:2 * FB, k * 128:(k + 1) * 128], NT,
                                    preferred_element_type=f32)
                st["gu"] = d if k == 0 else st["gu"] + d
                return {}

            def hidden():
                col = f_start(i) + lax.broadcasted_iota(i32, (16, FB), 1)
                g, u = _cols(st["gu"], FB)
                st["hid"] = jnp.where(col >= i * FB, g * _sigmoid(g) * u, 0.0).astype(bf16)
                return {0: _cols(st["hid"])}

            def down(n):
                cs = slice(n * 256, min((n + 1) * 256, D))
                y_vm[:, cs] += jnp.dot(st["hid"], wf_vm[i, 2 * FB:3 * FB, cs], preferred_element_type=f32)
                return {}

            def prefetch():
                @pl.when(i + 3 < NB)
                def _():
                    wq_copy(i + 3).start()
                    for cp in wf_copies(i + 2):
                        cp.start()

                @pl.when(i + 3 == NB)
                def _():
                    for cp in kv_copies(0, 0):
                        cp.start()

            tasks = {2 * c + 2: (lambda c=c: pick(c)) for c in range(C)}
            tasks[20] = gathered
            for k in range(KD):
                tasks[22 + k] = lambda k=k: gate_up(k)
            tasks[30] = hidden
            for n in range(3):
                tasks[32 + n] = lambda n=n: down(n)
            for t in range(S // T1):
                qproj(pl.ds(t * T1, T1), i + 1, zero,
                      lambda k, acc, t=t: tasks[t * KD + k]() if t * KD + k in tasks else {})
                if t == 0:
                    prefetch()
            return carry

        with scope("p1"):
            lax.fori_loop(0, NB - 1, phase1, 0)

        wo_copy().start()
        kbits = pltpu.bitcast(sel_vm[:, D:D + 128], i32)
        u = lax.shift_right_logical(kbits, 11) & 0xFFFF
        rsel = pltpu.bitcast(jnp.where(u >= 0x8000, u - 0x8000, 0xFFFF - u) << 16, f32)
        bsel = sel_vm[:, 0:D] + y_vm[0:8, :] * jnp.tile(_sigmoid(rsel), (1, KD))
        row16 = lax.broadcasted_iota(i32, (16, D), 0)
        for c in range(C):
            tok = (S - 1) - (kbits[c, 0] & (S - 1))
            grp = b_vm[token_group(tok), :].astype(f32)
            b_vm[token_group(tok), :] = jnp.where(row16 == (tok & 15), bsel[c:c + 1, :], grp).astype(bf16)

        NG = H // HB

        def phase2(g, carry):
            slot = g & 1
            kv_wait(slot)

            def prefetch():
                for cp in kv_copies(jnp.minimum(g + 1, NG - 1), 1 - slot):
                    cp.start()

            zero = lax.shift_right_logical(g, 8)

            class Tile:
                pass

            def qk(n):
                st = Tile()
                st.h, st.r = n // (S // TQ), pl.ds(n % (S // TQ) * TQ, TQ)
                st.s, st.mps, st.lp = [], [], None
                q = q_vm[g * HB + st.h, st.r, :]
                for c in range(NC):
                    s = _cols(lax.dot_general(q, kv_vm[slot, 0, st.h, c * CK:(c + 1) * CK, :], NT, preferred_element_type=f32))
                    mc = _fold(s, jnp.maximum)
                    st.mps.append(mc if c == 0 else jnp.maximum(st.mps[-1], mc))
                    st.s.append(s)
                st.m = jnp.broadcast_to(jnp.max(st.mps[-1], axis=-1, keepdims=True), (TQ, 128))
                return st

            def probs(st, c, deps):
                if len(deps) == 1:
                    mm = _after(st.m, [deps[0], st.lp], zero)
                    ps = [jnp.exp2(s - mm) for s in st.s[c]]
                    lc = _fold(ps, jnp.add)
                    st.lp = lc if st.lp is None else st.lp + lc
                else:
                    ps = []
                    for s, d in zip(st.s[c], deps):
                        p = jnp.exp2(s - _after(st.m, [d, st.lp], zero))
                        st.lp = p if st.lp is None else st.lp + p
                        ps.append(p)
                return jnp.concatenate(ps, axis=1).astype(bf16)

            NU = HB * (S // TQ)
            if kvpos == 0:
                prefetch()
            cur = qk(0)
            if kvpos == 1:
                prefetch()
            last = None
            for n in range(NU):
                nxt = qk(n + 1) if n + 1 < NU else None
                for c in range(NC):
                    if n == 0 and c == 0:
                        p = probs(cur, 0, [nxt.mps[j * NC // NJ] for j in range(NJ)])
                    else:
                        p = probs(cur, c, [last])
                    oc = jnp.dot(p, kv_vm[slot, 1, cur.h, c * CK:(c + 1) * CK, :], preferred_element_type=f32)
                    acc = oc if c == 0 else acc + oc
                    last = oc
                l = jnp.sum(cur.lp, axis=-1, keepdims=True)
                rl = pl.reciprocal(l, approx=True)
                rl = rl * (2.0 - l * rl)
                last = acc * rl
                o_vm[g * HB + cur.h, cur.r, :] = last.astype(bf16)
                cur = nxt
            return carry

        with scope("p2"):
            lax.fori_loop(0, NG, phase2, 0)
        kv_wait(NG & 1)
        wo_copy().wait()

        def phase3(i, carry):
            zero = lax.shift_right_logical(i, 8)
            for t in range(T3 // S3):
                n = i * (T3 // S3) + t
                r = pl.ds(pl.multiple_of(n * S3, S3), S3)
                for nn in range(KD):
                    cs = slice(nn * 128, (nn + 1) * 128)
                    b = b_vm[r, cs].astype(f32)
                    gate = b * _sigmoid(b)
                    gates = _rows(gate, 8)
                    acc = None
                    for kc in range(H // 4):
                        o = [o_vm[kc * 4 + a, r, :] for a in range(4)]
                        if 1 <= kc <= 4:
                            o[0] = _after_rows(o[0], {g: gates[2 * g:2 * g + 2] for g in range(kc - 1, S3 // 16, 4)}, zero)
                        d = jnp.dot(jnp.concatenate(o, axis=1), wo_vm[kc * 512:(kc + 1) * 512, cs], preferred_element_type=f32)
                        acc = d if acc is None else acc + d
                    out_vm[r, cs] = (x_vm[r, cs].astype(f32) + acc * gate).astype(bf16)
                    if nn in OC:
                        c0 = max([a + 1 for a in OC if a < nn], default=0)
                        cc = pl.ds(c0 * 128, (nn + 1 - c0) * 128)
                        pltpu.make_async_copy(out_vm.at[r, cc], out_hbm.at[r, cc], out_sem.at[0]).start()
            return carry

        with scope("p3"):
            lax.fori_loop(0, S // T3, phase3, 0)
        with scope("w_out"):
            pltpu.make_async_copy(out_vm, out_hbm, out_sem.at[0]).wait()

    def fn(A_x, A_k_cache, A_v_cache, A_wq, A_wo, B_x, B_w_r, B_w_gate, B_w_up, B_w_down):
        hbm = pl.BlockSpec(memory_space=pltpu.HBM)
        dma = pltpu.SemaphoreType.DMA
        out = pl.pallas_call(
            kernel,
            in_specs=[hbm, hbm, hbm, hbm, hbm, hbm, hbm, hbm, hbm],
            out_specs=hbm,
            out_shape=jax.ShapeDtypeStruct((S, D), bf16),
            scratch_shapes=[
                pltpu.VMEM((S, D), bf16), pltpu.VMEM((S, D), bf16), pltpu.VMEM((S, D), bf16),
                pltpu.VMEM((H, S, DH), bf16), pltpu.VMEM((H, S, DH), bf16),
                pltpu.VMEM((NB, D, 512), bf16), pltpu.VMEM((H * DH, D), bf16),
                pltpu.VMEM((NB - 1, 3 * FB, D), bf16),
                pltpu.VMEM((2, 2, HB, S, DH), bf16), pltpu.VMEM((S, D), bf16), pltpu.VMEM((D,), bf16),
                pltpu.VMEM((2, 8, 128), f32), pltpu.VMEM((8, D + 128), f32), pltpu.VMEM((16, D), f32),
                dma((NX,)), dma((4,)), dma((4,)), dma((1,)), dma((2,)), dma((1,)), dma((1,)),
            ],
            compiler_params=pltpu.CompilerParams(vmem_limit_bytes=110 * 2**20, flags=flags, disable_bounds_checks=nobc),
        )(A_x.reshape(S, D), A_k_cache.reshape(H, S, DH), A_v_cache.reshape(H, S, DH), A_wq, A_wo,
          B_w_r, B_w_gate.T, B_w_up.T, B_w_down)
        return out.reshape(1, S, D)
    return fn


@jax.jit
def pallas_recurrent_scan__mha_block_cached__moe_arch_mod__prompt_kernel(
    A_x, A_k_cache, A_v_cache, A_wq, A_wo, B_x, B_w_r, B_w_gate, B_w_up, B_w_down
):
    return _build(OC=(3,4))(A_x, A_k_cache, A_v_cache, A_wq, A_wo, B_x, B_w_r, B_w_gate, B_w_up, B_w_down)
```

```python
import contextlib
import jax, jax.numpy as jnp, numpy as np
from jax import lax
from jax.experimental import pallas as pl
from jax.experimental.pallas import tpu as pltpu

S, D, H, DH, F, C = 2048, 640, 32, 128, 1728, 8
f32, bf16, i32 = jnp.float32, jnp.bfloat16, jnp.int32
NT = (((1,), (1,)), ((), ()))
QSCALE = float(DH ** -0.5 * np.log2(np.e))
EPS_BF16 = 1.0013580322265625e-05
KD = D // 128


def _fold(xs, op):
    r = xs[0]
    for a in xs[1:]:
        r = op(r, a)
    return r


def _cols(a, w=128):
    return [a[:, j * w:(j + 1) * w] for j in range(a.shape[1] // w)]


def _rows(a, w):
    return [a[j * w:(j + 1) * w, :] for j in range(a.shape[0] // w)]


def _rb(a):
    return a.astype(bf16).astype(f32)


def _sigmoid(a):
    return pl.reciprocal(1.0 + jnp.exp(-a), approx=True)


def _dot(a, b):
    return jnp.dot(a, b, preferred_element_type=f32)


def _dot_nt(a, b):
    return lax.dot_general(a, b, NT, preferred_element_type=f32)


def _after(val, deps, zero):
    deps = [pltpu.bitcast(d, i32) for d in deps if d is not None]
    if not deps:
        return val
    return pltpu.bitcast(pltpu.bitcast(val, i32) | (_fold(deps, jnp.bitwise_or) & zero), val.dtype)


def _after_rows(lhs, deps, zero):
    if not deps:
        return lhs
    first = jnp.concatenate([_after(g, deps.get(n, []), zero) for n, g in enumerate(_rows(lhs[:, 0:128], 16))], axis=0)
    return first if lhs.shape[1] == 128 else jnp.concatenate([first, lhs[:, 128:]], axis=1)


def _build(XC=(2, 2, 4, 8), T0=128, DL=(2, 3, 4, 5, 7), PK=3, OC=(3, 4), SP=0, FC=0, DA=0, WD=0, TA=(), OM=0, TS=0, WP=9, UP=0, kvpos=1, prof=False, flags=None, nobc=False):
    TQ = 256
    CK = 512
    NP = H // 2
    NR = S // TQ
    NU = NR - 1
    FB = 128
    NX = len(XC)
    XO = [sum(XC[:i]) for i in range(NX + 1)]
    assert XO[-1] * T0 == S
    NC = S // CK
    scope = jax.named_scope if prof else (lambda name: contextlib.nullcontext())

    def kernel(x_hbm, k_hbm, v_hbm, wq_hbm, wo_hbm, wr_hbm, wg_hbm, wu_hbm, wd_hbm, out_hbm,
               x_vm, xn_vm, b_vm, q_vm, o_vm, s_vm, wq_vm, wo_vm, wf_vm, kv_vm, out_vm, wr_vm,
               key_vm, sel_vm, y_vm, x_sem, w_sem, kv_sem, out_sem):

        def x_copy(i):
            r = pl.ds(XO[i] * T0, XC[i] * T0)
            return pltpu.make_async_copy(x_hbm.at[r, :], x_vm.at[r, :], x_sem.at[i])

        def w_copies(part):
            sem = w_sem.at[part]
            p0, p1 = ((0, 2), (2, 3), (3, NP))[part]
            cps = [pltpu.make_async_copy(wq_hbm.at[:, pl.ds(p * 256, 256)], wq_vm.at[p], sem) for p in range(p0, p1)]
            if part > 0:
                r = (pl.ds(0, 1), pl.ds(1, NP - 1))[part - 1]
                cps.append(pltpu.make_async_copy(wo_hbm.at[r], wo_vm.at[r], sem))
                r = (pl.ds(0, FB), pl.ds(FB, F - FB))[part - 1]
                cps += [pltpu.make_async_copy(w.at[r, :], wf_vm.at[a, r, :], sem) for a, w in enumerate((wg_hbm, wu_hbm, wd_hbm))]
            return cps

        def kv_copies(g, slot):
            hs = pl.ds(g * 2, 2)
            return [pltpu.make_async_copy(k_hbm.at[hs], kv_vm.at[slot, 0], kv_sem.at[slot]),
                    pltpu.make_async_copy(v_hbm.at[hs], kv_vm.at[slot, 1], kv_sem.at[slot])]

        def kv_wait(slot):
            pltpu.make_async_copy(kv_vm.at[slot], kv_vm.at[slot], kv_sem.at[slot]).wait()

        wr_copy = pltpu.make_async_copy(wr_hbm, wr_vm, out_sem.at[1])
        wr_copy.start()
        x_copy(0).start()
        for cp in w_copies(0):
            cp.start()
        s_vm[...] = jnp.zeros_like(s_vm)
        y_vm[...] = jnp.zeros_like(y_vm)
        sel_vm[...] = jnp.zeros_like(sel_vm)
        wr_copy.wait()
        x_copy(0).wait()
        x_copy(1).start()
        wr = wr_vm[...].astype(f32).reshape(1, D)
        zero0 = lax.shift_right_logical(pltpu.bitcast(jnp.broadcast_to(wr[:, 0:128], (8, 128)), i32)[0, 0] & 1, 1)
        lane = lax.broadcasted_iota(i32, (8, 128), 1)
        sub = lax.broadcasted_iota(i32, (8, 128), 0)
        rpack = [jnp.zeros((8, 128), f32), jnp.zeros((8, 128), f32)]

        def layernorm(r0, n, start=None):
            r = pl.ds(r0, n)
            x = x_vm[r, :].astype(f32)
            if start is not None:
                xs = _cols(x)
                x = jnp.concatenate([_after(xs[0], [start], zero0)] + xs[1:], axis=1)
            mean = jnp.sum(x, axis=-1, keepdims=True) * (1.0 / D)
            yield mean
            shift = _rb(mean)
            d = x - shift
            var = jnp.sum(d * d, axis=-1, keepdims=True) * (1.0 / D) - (mean - shift) * (mean - shift)
            yield var
            inv = pl.reciprocal(_rb(jnp.sqrt(_rb(_rb(var) + EPS_BF16))), approx=True)
            yield inv
            xn = d * inv
            xnb = xn.astype(bf16)
            xn_vm[r, :] = xnb
            b_vm[r, :] = xnb
            part = _fold(_cols(xn * wr), jnp.add)
            yield part
            score = jnp.broadcast_to(jnp.sum(part, axis=-1, keepdims=True), (n, 128))
            packed = []
            for a, sc in enumerate(_rows(score, 8)):
                g = r0 // 8 + a
                rpack[g // 128] = jnp.where(lane == g % 128, sc, rpack[g // 128])
                packed.append(rpack[g // 128])
            yield jnp.concatenate(packed, axis=0)

        NT0 = S // T0
        first = XC[0]
        for _ in layernorm(0, first * T0):
            pass
        with scope("w_wq0"):
            for cp in w_copies(0):
                cp.wait()
        x_copy(2).start()
        running = {}
        prev = None
        for n in range(NT0):
            t = n + 1
            waits = []
            if first <= t < NT0 and t in XO:
                i = XO.index(t)
                waits.append(x_copy(i).wait)
                if i + 2 < NX:
                    waits.append(x_copy(i + 2).start)
                if i + 2 == NX:
                    waits += [cp.start for cp in kv_copies(0, 0) + w_copies(1)]
            for a, w in enumerate(waits):
                with scope(f"w_{n}_{a}"):
                    w()
            if first <= t < NT0:
                gen = layernorm(t * T0, T0, None if waits else prev)
                for a in DL:
                    running.setdefault(n * KD + a, []).append(gen)
            r = pl.ds(n * T0, T0)
            acc = None
            for k in range(KD):
                ks = slice(k * 128, (k + 1) * 128)
                vs = [_rows(jnp.broadcast_to(next(gen), (T0, 128)), 8) for gen in running.pop(n * KD + k, [])]
                deps = {a: [v[2 * a + 1] for v in vs] for a in range(T0 // 16)} if vs else {}
                d = _dot(_after_rows(xn_vm[r, ks], deps, zero0), jnp.concatenate([wq_vm[0, ks, :], wq_vm[1, ks, :]], axis=1))
                acc = d if acc is None else acc + d
                if k == PK:
                    prev = d[:, 0:128]
            for c, qc in enumerate(_cols(acc * QSCALE)):
                q_vm[c, r, :] = qc.astype(bf16)
        assert not running
        for a in range(2):
            rb = _rb(rpack[a])
            rb = jnp.where(rb == 0.0, 0.0, rb)
            bits = lax.shift_right_logical(pltpu.bitcast(rb, i32), 16)
            u = jnp.where(bits >= 0x8000, 0xFFFF - bits, bits + 0x8000)
            u = jnp.where(rb != rb, 0, u)
            idx = a * 1024 + lane * 8 + sub
            key_vm[a] = pltpu.bitcast((1 << 29) + u * 2048 + (S - 1 - idx), f32)
        with scope("w_w1"):
            for cp in w_copies(1):
                cp.wait()
        for cp in w_copies(2):
            cp.start()

        def token_group(tok):
            return pl.ds(pl.multiple_of((tok >> 4) << 4, 16), 16)

        def step(g, carry):
            slot = g & 1
            kv_wait(slot)

            @pl.when(g == 1)
            def _():
                for cp in w_copies(2):
                    cp.wait()
                row16 = lax.broadcasted_iota(i32, (16, D), 0)
                kbits = pltpu.bitcast(key_vm[2], i32)
                xsel = jnp.zeros((16, D), f32)
                for c in range(C):
                    tok = (S - 1) - (kbits[c, 0] & (S - 1))
                    grp = xn_vm[token_group(tok), :].astype(f32)
                    rowv = jnp.sum(jnp.where(row16 == (tok & 15), grp, 0.0), axis=0, keepdims=True)
                    xsel = jnp.where(row16 == c, rowv, xsel)
                sel_vm[...] = xsel.astype(bf16)

            zero = lax.shift_right_logical(g, 8)

            st = dict(k0=key_vm[0], k1=key_vm[1], keys=jnp.zeros((8, 128), f32))
            f0 = pl.multiple_of(jnp.clip((g - 1) * FB, 0, F - FB), 64)

            def pick(c):
                k0, k1 = st["k0"], st["k1"]
                mx = jnp.max(jnp.max(jnp.maximum(k0, k1), axis=1, keepdims=True), axis=0, keepdims=True)
                st["k0"] = jnp.where(k0 == mx, 0.0, k0)
                st["k1"] = jnp.where(k1 == mx, 0.0, k1)
                st["keys"] = jnp.where(sub == c, mx, st["keys"])
                if c == C - 1:
                    key_vm[2] = st["keys"]
                return {0: [st["keys"]]}

            def gate_up(k):
                ks = slice(k * 256, min((k + 1) * 256, D))
                w = jnp.concatenate([wf_vm[0, pl.ds(f0, FB), ks], wf_vm[1, pl.ds(f0, FB), ks]], axis=0)
                d = _dot_nt(sel_vm[:, ks], w)
                st["gu"] = d if k == 0 else st["gu"] + d
                return {}

            def hidden():
                col = f0 + lax.broadcasted_iota(i32, (16, FB), 1)
                gt, up = _cols(st["gu"], FB)
                st["hid"] = jnp.where(col >= jnp.where(g == 0, F, (g - 1) * FB), gt * _sigmoid(gt) * up, 0.0).astype(bf16)
                return {0: [st["hid"]]}

            def down(n):
                cs = slice(n * 512, min((n + 1) * 512, D))
                y_vm[:, cs] += _dot(st["hid"], wf_vm[2, pl.ds(f0, FB), cs])
                return {}

            tasks = {(1, 0): lambda: [pick(c) for c in range(4)][-1], (2, 0): lambda: [pick(c) for c in range(4, 8)][-1]}
            if TS == 0:
                for k in range(3):
                    tasks[4, k] = lambda k=k: gate_up(k)
                tasks[5, 0] = hidden
                tasks[6, 0] = lambda: down(0)
                tasks[6, 1] = lambda: down(1)
            side = lambda j, a: tasks[j, a]() if (j, a) in tasks else {}

            def unit(j):
                u = g * NU + j
                return u >> 3, pl.multiple_of((u & 7) * TQ, TQ)

            def q_unit(j):
                p, r0 = unit(j)
                r = pl.ds(r0, TQ)
                ds = [_dot(_after_rows(xn_vm[r, a * 256:(a + 1) * 256], side(j, a), zero), wq_vm[p + 2, a * 256:(a + 1) * 256, :])
                      for a in range(2)]
                last = [_dot(_after_rows(xn_vm[pl.ds(r0 + a * 128, 128), 512:D], side(j, 2 + a), zero), wq_vm[p + 2, 512:D, :])
                        for a in range(2)]
                q = (ds[0] + ds[1] + jnp.concatenate(last, axis=0)) * QSCALE
                for c, qc in enumerate(_cols(q)):
                    q_vm[2 * p + 4 + c, r, :] = qc.astype(bf16)
                return ds

            def o_load(j):
                p, r0 = unit(j)
                return jnp.concatenate([o_vm[2 * p + c, pl.ds(r0, TQ), :] for c in range(2)], axis=1)

            def o_unit(j, o):
                p, r0 = unit(j)
                if OM == 0:
                    ds = [_dot(o, wo_vm[p, :, a * 256:(a + 1) * 256]) for a in range(2)]
                else:
                    ds = [_dot(o[:, 0:128], wo_vm[p, 0:128, 0:512])
                          + _dot(o[:, 128:256], wo_vm[p, 128:256, 0:512])]
                ds.append(jnp.concatenate([_dot(oa, wo_vm[p, :, 512:D]) for oa in _rows(o, 128)], axis=0))
                s_vm[pl.ds(r0, TQ), :] += jnp.concatenate(ds, axis=1)
                return ds[WD][:, 0:128]

            late = []

            def flush(dep):
                tl, ol = late.pop()
                deps = {} if dep is None else {a: [d] for a, d in enumerate(_rows(dep, 8)[::2])}
                o_vm[g * 2 + tl.h, tl.r, :] = _after_rows(ol, deps, zero)

            class Tile:
                pass

            def scores(n):
                t = Tile()
                t.h, t.r = n // NR, pl.ds(n % NR * TQ, TQ)
                t.s, t.mps, t.lp = [], [], None
                q = q_vm[g * 2 + t.h, t.r, :]
                t.u = q_unit(n) if n < NU else None
                for c in range(NC):
                    s = _cols(_dot_nt(q, kv_vm[slot, 0, t.h, c * CK:(c + 1) * CK, :]))
                    mc = _fold(s, jnp.maximum)
                    t.mps.append(mc if c == 0 else jnp.maximum(t.mps[-1], mc))
                    t.s.append(s)
                    if c == FC and late:
                        flush(s[0])
                t.m = jnp.broadcast_to(jnp.max(t.mps[-1], axis=-1, keepdims=True), (TQ, 128))
                return t

            def probs(t, c, deps):
                if len(deps) == 1:
                    mm = _after(t.m, [deps[0], t.lp], zero)
                    ps = [jnp.exp2(s - mm) for s in t.s[c]]
                    lc = _fold(ps, jnp.add)
                    t.lp = lc if t.lp is None else t.lp + lc
                else:
                    ps = []
                    for s, d in zip(t.s[c], deps):
                        p = jnp.exp2(s - _after(t.m, [d, t.lp], zero))
                        t.lp = p if t.lp is None else t.lp + p
                        ps.append(p)
                return jnp.concatenate(ps, axis=1).astype(bf16)

            cur = scores(0)
            for cp in kv_copies(jnp.minimum(g + 1, NP - 1), 1 - slot):
                cp.start()
            last = None
            for n in range(2 * NR):
                nxt = scores(n + 1) if n + 1 < 2 * NR else None
                for c in range(NC):
                    if n == 0 and c == 0:
                        p = probs(cur, 0, nxt.mps if SP == 0 else [nxt.u[SP - 1][:, 0:128]])
                    else:
                        p = probs(cur, c, [acc if c in TA else last])
                    last = _dot(p, kv_vm[slot, 1, cur.h, c * CK:(c + 1) * CK, :])
                    acc = last if c == 0 else acc + last
                l = jnp.sum(cur.lp, axis=-1, keepdims=True)
                rl = pl.reciprocal(l, approx=True)
                last = acc * (rl * (2.0 - l * rl))
                wd = o_unit(n - WP, o_load(n - WP)) if 0 <= n - WP < NU else None
                if n + 1 < 2 * NR and (DA or n >= WP):
                    late.append((cur, last.astype(bf16)))
                    if n + 2 == 2 * NR:
                        flush(wd)
                else:
                    late.append((cur, last.astype(bf16)))
                    flush(wd if n >= WP else None)
                cur = nxt
            return carry

        with scope("loop"):
            lax.fori_loop(0, NP, step, 0)
        kv_wait(NP & 1)

        kbits = pltpu.bitcast(key_vm[2], i32)
        u = lax.shift_right_logical(kbits, 11) & 0xFFFF
        rsel = pltpu.bitcast(jnp.where(u >= 0x8000, u - 0x8000, 0xFFFF - u) << 16, f32)
        bsel = sel_vm[...].astype(f32)[0:8, :] + y_vm[0:8, :] * jnp.tile(_sigmoid(rsel), (1, KD))
        row16 = lax.broadcasted_iota(i32, (16, D), 0)
        for c in range(C):
            tok = (S - 1) - (kbits[c, 0] & (S - 1))
            grp = b_vm[token_group(tok), :].astype(f32)
            b_vm[token_group(tok), :] = jnp.where(row16 == (tok & 15), bsel[c:c + 1, :], grp).astype(bf16)

        with scope("epi"):
            for n in range(NR):
                r = pl.ds(n * TQ, TQ)
                for nn in range(KD):
                    cs = slice(nn * 128, (nn + 1) * 128)
                    o = jnp.concatenate([o_vm[H - 4 + a, r, :] for a in range(4)], axis=1)
                    s = s_vm[r, cs] + _dot(o, jnp.concatenate([wo_vm[NP - 2, :, cs], wo_vm[NP - 1, :, cs]], axis=0))
                    b = b_vm[r, cs].astype(f32)
                    out_vm[r, cs] = (x_vm[r, cs].astype(f32) + s * (b * _sigmoid(b))).astype(bf16)
                    oc = OC if n == NR - 1 else (KD - 1,)
                    if nn in oc:
                        c0 = max([a + 1 for a in oc if a < nn], default=0)
                        cc = pl.ds(c0 * 128, (nn + 1 - c0) * 128)
                        pltpu.make_async_copy(out_vm.at[r, cc], out_hbm.at[r, cc], out_sem.at[0]).start()
        with scope("w_out"):
            pltpu.make_async_copy(out_vm, out_hbm, out_sem.at[0]).wait()

    def fn(A_x, A_k_cache, A_v_cache, A_wq, A_wo, B_x, B_w_r, B_w_gate, B_w_up, B_w_down):
        hbm = pl.BlockSpec(memory_space=pltpu.HBM)
        dma = pltpu.SemaphoreType.DMA
        out = pl.pallas_call(
            kernel,
            in_specs=[hbm] * 9,
            out_specs=hbm,
            out_shape=jax.ShapeDtypeStruct((S, D), bf16),
            scratch_shapes=[
                pltpu.VMEM((S, D), bf16), pltpu.VMEM((S, D), bf16), pltpu.VMEM((S, D), bf16),
                pltpu.VMEM((H, S, DH), bf16), pltpu.VMEM((H, S, DH), bf16), pltpu.VMEM((S, D), f32),
                pltpu.VMEM((NP, D, 256), bf16), pltpu.VMEM((NP, 256, D), bf16), pltpu.VMEM((3, F, D), bf16),
                pltpu.VMEM((2, 2, 2, S, DH), bf16), pltpu.VMEM((S, D), bf16), pltpu.VMEM((D,), bf16),
                pltpu.VMEM((3, 8, 128), f32), pltpu.VMEM((16, D), bf16), pltpu.VMEM((16, D), f32),
                dma((NX,)), dma((3,)), dma((2,)), dma((2,)),
            ],
            compiler_params=pltpu.CompilerParams(vmem_limit_bytes=110 * 2**20, flags=flags, disable_bounds_checks=nobc),
        )(A_x.reshape(S, D), A_k_cache.reshape(H, S, DH), A_v_cache.reshape(H, S, DH), A_wq, A_wo.reshape(NP, 256, D),
          B_w_r, B_w_gate.T, B_w_up.T, B_w_down)
        return out.reshape(1, S, D)
    return fn


@jax.jit
def pallas_recurrent_scan__mha_block_cached__moe_arch_mod__prompt_kernel(
    A_x, A_k_cache, A_v_cache, A_wq, A_wo, B_x, B_w_r, B_w_gate, B_w_up, B_w_down
):
    return _build(WD=1)(A_x, A_k_cache, A_v_cache, A_wq, A_wo, B_x, B_w_r, B_w_gate, B_w_up, B_w_down)
```

```python
import contextlib
import jax, jax.numpy as jnp, numpy as np
from jax import lax
from jax.experimental import pallas as pl
from jax.experimental.pallas import tpu as pltpu

S, D, H, DH, F, C = 2048, 640, 32, 128, 1728, 8
f32, bf16, i32 = jnp.float32, jnp.bfloat16, jnp.int32
NT = (((1,), (1,)), ((), ()))
QSCALE = float(DH ** -0.5 * np.log2(np.e))
EPS_BF16 = 1.0013580322265625e-05
KD = D // 128


def _fold(xs, op):
    r = xs[0]
    for a in xs[1:]:
        r = op(r, a)
    return r


def _reduce(acc, xs, op, mode):
    if mode >= 2:
        return _fold(([] if acc is None else [acc]) + (xs if mode == 2 else xs[::-1]), op)
    r = _fold(xs, op) if mode == 0 else op(op(xs[0], xs[1]), op(xs[2], xs[3]))
    return r if acc is None else op(acc, r)


def _cols(a, w=128):
    return [a[:, j * w:(j + 1) * w] for j in range(a.shape[1] // w)]


def _rows(a, w):
    return [a[j * w:(j + 1) * w, :] for j in range(a.shape[0] // w)]


def _rb(a):
    return a.astype(bf16).astype(f32)


def _sigmoid(a):
    return pl.reciprocal(1.0 + jnp.exp(-a), approx=True)


def _dot(a, b):
    return lax.dot_general(a, b, (((1,), (0,)), ((), ())), preferred_element_type=f32)


def _dot_nt(a, b):
    return lax.dot_general(a, b, NT, preferred_element_type=f32)


def _after(val, deps, zero):
    deps = [pltpu.bitcast(d, i32) for d in deps if d is not None]
    if not deps:
        return val
    return pltpu.bitcast(pltpu.bitcast(val, i32) | (_fold(deps, jnp.bitwise_or) & zero), val.dtype)


def _after_rows(lhs, deps, zero):
    if not deps:
        return lhs
    first = jnp.concatenate([_after(g, deps.get(n, []), zero) for n, g in enumerate(_rows(lhs[:, 0:128], 16))], axis=0)
    return first if lhs.shape[1] == 128 else jnp.concatenate([first, lhs[:, 128:]], axis=1)


def _build(XC=(2, 2, 4, 8), T0=128, DL=(2, 3, 4, 5, 8), PK=3, OC=(1, 2, 3, 4), SP=2, FC=1, DA=0, WD=1, LT=0, NW=1, T0R=0, GT=1, FM=1, FS=0, CH=1, F32=0, PU=(1, 2), GU=(4, 5, 6), QM=1, FP=(0, 1, 2, 0, 1), TA=(), OM=1, TS=0, WP=9, UP=0, kvpos=0, prof=False, flags=None, nobc=False):
    TQ = 256
    CK = 512
    NP = H // 2
    NR = S // TQ
    NU = NR - 1
    FB = 128
    NX = len(XC)
    XO = [sum(XC[:i]) for i in range(NX + 1)]
    assert XO[-1] * T0 == S and DL[3] <= KD
    NC = S // CK
    scope = jax.named_scope if prof else (lambda name: contextlib.nullcontext())

    def kernel(x_hbm, k_hbm, v_hbm, wq_hbm, wo_hbm, wr_hbm, wg_hbm, wu_hbm, wd_hbm, out_hbm,
               x_vm, xn_vm, q_vm, o_vm, s_vm, wq_vm, wo_vm, wf_vm, kv_vm, out_vm, wr_vm,
               key_vm, sel_vm, y_vm, x_sem, w_sem, kv_sem, out_sem):

        def x_copy(i):
            r = pl.ds(XO[i] * T0, XC[i] * T0)
            return pltpu.make_async_copy(x_hbm.at[r, :], x_vm.at[r, :], x_sem.at[i % 2])

        def w_copies(part):
            sem = w_sem.at[part % 2]
            p0, p1 = ((0, 2), (2, 3), (3, NP))[part]
            cps = [pltpu.make_async_copy(wq_hbm.at[:, pl.ds(p * 256, 256)], wq_vm.at[p], sem) for p in range(p0, p1)]
            if part > 0:
                r = (pl.ds(0, 1), pl.ds(1, NP - 1))[part - 1]
                cps.append(pltpu.make_async_copy(wo_hbm.at[r], wo_vm.at[r], sem))
                r = (pl.ds(0, FB), pl.ds(FB, F - FB))[part - 1]
                cps += [pltpu.make_async_copy(w.at[r, :], wf_vm.at[a, r, :], sem) for a, w in enumerate((wg_hbm, wu_hbm, wd_hbm))]
            return cps

        def kv_copies(g, slot):
            hs = pl.ds(g * 2, 2)
            return [pltpu.make_async_copy(k_hbm.at[hs], kv_vm.at[slot, 0], kv_sem.at[0]),
                    pltpu.make_async_copy(v_hbm.at[hs], kv_vm.at[slot, 1], kv_sem.at[0])]

        def kv_wait(slot):
            pltpu.make_async_copy(kv_vm.at[slot], kv_vm.at[slot], kv_sem.at[0]).wait()

        wr_copy = pltpu.make_async_copy(wr_hbm, wr_vm, out_sem.at[0])
        wr_copy.start()
        x_copy(0).start()
        for cp in w_copies(0):
            cp.start()
        s_vm[...] = jnp.zeros_like(s_vm)
        y_vm[...] = jnp.zeros_like(y_vm)
        sel_vm[...] = jnp.zeros_like(sel_vm)
        wr_copy.wait()
        x_copy(0).wait()
        x_copy(1).start()
        wr = wr_vm[...].astype(f32).reshape(1, D)
        zero0 = lax.shift_right_logical(pltpu.bitcast(jnp.broadcast_to(wr[:, 0:128], (8, 128)), i32)[0, 0] & 1, 1)
        lane = lax.broadcasted_iota(i32, (8, 128), 1)
        sub = lax.broadcasted_iota(i32, (8, 128), 0)
        rpack = [jnp.zeros((8, 128), f32), jnp.zeros((8, 128), f32)]

        def layernorm(r0, n, start=None):
            r = pl.ds(r0, n)
            x = x_vm[r, :].astype(f32)
            if start is not None:
                xs = _cols(x)
                x = jnp.concatenate([_after(xs[0], [start], zero0)] + xs[1:], axis=1)
            mean = jnp.sum(x, axis=-1, keepdims=True) * (1.0 / D)
            yield mean
            shift = _rb(mean)
            d = x - shift
            var = jnp.maximum(jnp.sum(d * d, axis=-1, keepdims=True) * (1.0 / D) - (mean - shift) * (mean - shift), 0.0)
            yield var
            inv = pl.reciprocal(_rb(jnp.sqrt(_rb(_rb(var) + EPS_BF16))), approx=True)
            yield inv
            xn = d * inv
            xnb = xn.astype(bf16)
            xn_vm[r, :] = xnb
            part = _fold(_cols(xn * wr), jnp.add)
            yield part
            score = jnp.broadcast_to(jnp.sum(part, axis=-1, keepdims=True), (n, 128))
            packed = []
            for a, sc in enumerate(_rows(score, 8)):
                g = r0 // 8 + a
                rpack[g // 128] = jnp.where(lane == g % 128, sc, rpack[g // 128])
                packed.append(rpack[g // 128])
            yield jnp.concatenate(packed, axis=0)

        NT0 = S // T0
        first = XC[0]
        for _ in layernorm(0, first * T0):
            pass
        with scope("w_wq0"):
            for cp in w_copies(0):
                cp.wait()
        x_copy(2).start()
        running = {}
        prev = None
        for n in range(NT0):
            t = n + 1
            if first <= t < NT0:
                if t in XO:
                    i = XO.index(t)
                    with scope(f"w_x{i}"):
                        x_copy(i).wait()
                    if i + 2 < NX:
                        x_copy(i + 2).start()
                    if i + 2 == NX:
                        for cp in kv_copies(0, 0) + w_copies(1):
                            cp.start()
                    prev = None
                gen = layernorm(t * T0, T0, prev)
                for a in DL:
                    running.setdefault(n * KD + a, []).append(gen)
            if n == NT0 - 2:
                for cp in w_copies(2):
                    cp.start()
            r = pl.ds(n * T0, T0)
            acc = None
            for k in range(KD):
                ks = slice(k * 128, (k + 1) * 128)
                vs = [_rows(jnp.broadcast_to(next(gen), (T0, 128)), 8) for gen in running.pop(n * KD + k, [])]
                deps = {a: [v[2 * a + LT] for v in vs] for a in range(T0 // 16)} if vs else {}
                d = _dot(_after_rows(xn_vm[r, ks], deps, zero0), jnp.concatenate([wq_vm[0, ks, :], wq_vm[1, ks, :]], axis=1))
                acc = d if acc is None else acc + d
                if k == PK:
                    prev = d[:, 0:128]
            for c, qc in enumerate(_cols(acc * QSCALE)):
                q_vm[c, r, :] = qc.astype(bf16)
        assert not running
        for a in range(2):
            rb = _rb(rpack[a])
            rb = jnp.where(rb == 0.0, 0.0, rb)
            bits = lax.shift_right_logical(pltpu.bitcast(rb, i32), 16)
            u = jnp.where(bits >= 0x8000, 0xFFFF - bits, bits + 0x8000)
            u = jnp.where(rb != rb, 0, u)
            idx = a * 1024 + lane * 8 + sub
            key_vm[a] = pltpu.bitcast((1 << 29) + u * 2048 + (S - 1 - idx), f32)
        with scope("w_w1"):
            for cp in w_copies(1):
                cp.wait()

        def token_group(tok):
            return pl.ds(pl.multiple_of((tok >> 4) << 4, 16), 16)

        def step(g, carry):
            slot = g & 1
            kv_wait(slot)

            @pl.when(g == 1)
            def _():
                for cp in w_copies(2):
                    cp.wait()
                row16 = lax.broadcasted_iota(i32, (16, D), 0)
                kbits = pltpu.bitcast(key_vm[2], i32)
                xsel = jnp.zeros((16, D), f32)
                for c in range(C):
                    tok = (S - 1) - (kbits[c, 0] & (S - 1))
                    grp = xn_vm[token_group(tok), :].astype(f32)
                    rowv = jnp.sum(jnp.where(row16 == (tok & 15), grp, 0.0), axis=0, keepdims=True)
                    xsel = jnp.where(row16 == c, rowv, xsel)
                sel_vm[...] = xsel[0:8, :]

            zero = lax.shift_right_logical(g, 8)

            st = dict(k0=key_vm[0], k1=key_vm[1], keys=jnp.zeros((8, 128), f32))
            f0 = pl.multiple_of(jnp.clip((g - 1) * FB, 0, F - FB), 64)

            def pick(c):
                k0, k1 = st["k0"], st["k1"]
                mx = jnp.max(jnp.max(jnp.maximum(k0, k1), axis=1, keepdims=True), axis=0, keepdims=True)
                st["k0"] = jnp.where(k0 == mx, 0.0, k0)
                st["k1"] = jnp.where(k1 == mx, 0.0, k1)
                st["keys"] = jnp.where(sub == c, mx, st["keys"])
                if c == C - 1:
                    key_vm[2] = st["keys"]
                return {0: [st["keys"]]}

            lhs8 = (lambda a: a) if F32 else (lambda a: a.astype(bf16))

            def gate_up(k):
                ks = slice(k * 256, min((k + 1) * 256, D))
                w = jnp.concatenate([wf_vm[0, pl.ds(f0, FB), ks], wf_vm[1, pl.ds(f0, FB), ks]], axis=0)
                d = _dot_nt(lhs8(sel_vm[:, ks]), w)
                st["gu"] = d if k == 0 else st["gu"] + d
                return {}

            def hidden():
                col = f0 + lax.broadcasted_iota(i32, (8, FB), 1)
                gt, up = _cols(st["gu"], FB)
                st["hid"] = _rb(jnp.where(col >= jnp.where(g == 0, F, (g - 1) * FB), gt * _sigmoid(gt) * up, 0.0))
                return {0: [st["hid"]]}

            def down(n):
                cs = slice(n * 512, min((n + 1) * 512, D))
                if F32 == 2 and n == 1:
                    d = _dot(st["hid"], wf_vm[2, pl.ds(f0, FB), 384:D])
                    y_vm[:, cs] += _after(d[:, 128:256], [d[:, 0:128]], zero)
                else:
                    y_vm[:, cs] += _dot(lhs8(st["hid"]), wf_vm[2, pl.ds(f0, FB), cs])
                return {}

            tasks = {}
            for c in range(C):
                tasks.setdefault((PU[c // 4], 0), []).append(lambda c=c: pick(c))
            for k in range(3):
                tasks.setdefault((GU[0], FP[k]), []).append(lambda k=k: gate_up(k))
            tasks.setdefault((GU[1], 0), []).append(hidden)
            for k in range(2):
                tasks.setdefault((GU[2], FP[3 + k]), []).append(lambda k=k: down(k))
            side = lambda j, a: ([{}] + [f() for f in tasks.get((j, a), [])])[-1]

            def unit(j):
                u = g * NU + j
                return u >> 3, pl.multiple_of((u & 7) * TQ, TQ)

            def q_unit(j):
                p, r0 = unit(j)
                r = pl.ds(r0, TQ)
                tail = lambda: [_dot(_after_rows(xn_vm[pl.ds(r0 + a * 128, 128), 512:D], side(j, 2 + a), zero), wq_vm[p + 2, 512:D, :])
                                for a in range(2)]
                if QM & 2:
                    last = tail()
                if QM & 1:
                    ds = [_dot(_after_rows(xn_vm[r, 0:512], side(j, a), zero), wq_vm[p + 2, 0:512, a * 128:(a + 1) * 128]) for a in range(2)]
                    main = jnp.concatenate(ds, axis=1)
                else:
                    ds = [_dot(_after_rows(xn_vm[r, a * 256:(a + 1) * 256], side(j, a), zero), wq_vm[p + 2, a * 256:(a + 1) * 256, :])
                          for a in range(2)]
                    main = ds[0] + ds[1]
                if not QM & 2:
                    last = tail()
                q = (main + jnp.concatenate(last, axis=0)) * QSCALE
                for c, qc in enumerate(_cols(q)):
                    q_vm[2 * p + 4 + c, r, :] = qc.astype(bf16)
                return ds

            def o_load(j):
                p, r0 = unit(j)
                return jnp.concatenate([o_vm[2 * p + c, pl.ds(r0, TQ), :] for c in range(2)], axis=1)

            def o_unit(j, o):
                p, r0 = unit(j)
                if OM == 0:
                    ds = [_dot(o, wo_vm[p, :, a * 256:(a + 1) * 256]) for a in range(2)]
                else:
                    ds = [_dot(o[:, 0:128], wo_vm[p, 0:128, 0:512])
                          + _dot(o[:, 128:256], wo_vm[p, 128:256, 0:512])]
                ds.append(jnp.concatenate([_dot(oa, wo_vm[p, :, 512:D]) for oa in _rows(o, 128)], axis=0))
                s_vm[pl.ds(r0, TQ), :] += jnp.concatenate(ds, axis=1)
                return ds[WD][:, 0:128]

            late = []

            def flush(dep):
                tl, ol = late.pop()
                deps = {} if dep is None else {a: [d] for a, d in enumerate(_rows(dep, 8)[::2])}
                o_vm[g * 2 + tl.h, tl.r, :] = _after_rows(ol, deps, zero)

            class Tile:
                pass

            def scores(n):
                t = Tile()
                t.h, t.r = n // NR, pl.ds(n % NR * TQ, TQ)
                t.s, t.mps, t.lp = [], [], None
                q = q_vm[g * 2 + t.h, t.r, :]
                t.u = q_unit(n) if n < NU else None
                for c in range(NC):
                    s = _cols(_dot_nt(q, kv_vm[slot, 0, t.h, c * CK:(c + 1) * CK, :]))
                    t.mps.append(_reduce(t.mps[-1] if c else None, s, jnp.maximum, FM))
                    t.s.append(s)
                    if c == FC and late:
                        flush(s[0])
                t.m = jnp.broadcast_to(jnp.max(t.mps[-1], axis=-1, keepdims=True), (TQ, 128))
                return t

            def probs(t, c, deps):
                if len(deps) < NC:
                    mm = _after(t.m, deps + [t.lp], zero)
                    ps = [jnp.exp2(s - mm) for s in t.s[c]]
                    t.lp = _reduce(t.lp, ps, jnp.add, FS)
                    if CH:
                        t.m = mm
                else:
                    ps = []
                    for s, d in zip(t.s[c], deps):
                        p = jnp.exp2(s - _after(t.m, [d, t.lp], zero))
                        t.lp = p if t.lp is None else t.lp + p
                        ps.append(p)
                return jnp.concatenate(ps, axis=1).astype(bf16)

            cur = scores(0)
            last = None
            for n in range(2 * NR):
                if n == kvpos:
                    for cp in kv_copies(jnp.minimum(g + 1, NP - 1), 1 - slot):
                        cp.start()
                nxt = scores(n + 1) if n + 1 < 2 * NR else None
                for c in range(NC):
                    if n == 0 and c == 0:
                        p = probs(cur, 0, nxt.mps if SP == 0 else [nxt.u[SP - 1][:, 0:128]])
                    else:
                        p = probs(cur, c, [raw] if c == 0 and T0R and n else [last, done] if c == 1 and T0R and n else [acc if c in TA else last])
                    last = _dot(p, kv_vm[slot, 1, cur.h, c * CK:(c + 1) * CK, :])
                    acc = last if c == 0 else acc + last
                l = jnp.sum(cur.lp, axis=-1, keepdims=True)
                rl = pl.reciprocal(l, approx=True)
                raw = last
                last = acc * (rl * (2.0 - l * rl) if NW else rl)
                done = last
                wd = o_unit(n - WP, o_load(n - WP)) if 0 <= n - WP < NU else None
                if n + 1 < 2 * NR and (DA or n >= WP):
                    late.append((cur, last.astype(bf16)))
                    if n + 2 == 2 * NR:
                        flush(wd)
                else:
                    late.append((cur, last.astype(bf16)))
                    flush(wd if n >= WP else None)
                cur = nxt
            return carry

        with scope("loop"):
            lax.fori_loop(0, NP, step, 0)
        kv_wait(NP & 1)

        kbits = pltpu.bitcast(key_vm[2], i32)
        u = lax.shift_right_logical(kbits, 11) & 0xFFFF
        rsel = pltpu.bitcast(jnp.where(u >= 0x8000, u - 0x8000, 0xFFFF - u) << 16, f32)
        bsel = sel_vm[...] + y_vm[...] * jnp.tile(_sigmoid(rsel), (1, KD))
        row16 = lax.broadcasted_iota(i32, (16, D), 0)
        for c in range(C):
            tok = (S - 1) - (kbits[c, 0] & (S - 1))
            grp = xn_vm[token_group(tok), :].astype(f32)
            xn_vm[token_group(tok), :] = jnp.where(row16 == (tok & 15), bsel[c:c + 1, :], grp).astype(bf16)

        with scope("epi"):
            for n in range(NR):
                r = pl.ds(n * TQ, TQ)
                for nn in range(KD):
                    cs = slice(nn * 128, (nn + 1) * 128)
                    b = xn_vm[r, cs].astype(f32)
                    gate = b * _sigmoid(b)
                    o = jnp.concatenate([o_vm[H - 4 + a, r, :] for a in range(4)], axis=1)
                    if GT and n > 0:
                        o = _after_rows(o, {a: [d] for a, d in enumerate(_rows(gate, 8)[1::2])}, zero0)
                    s = s_vm[r, cs] + _dot(o, jnp.concatenate([wo_vm[NP - 2, :, cs], wo_vm[NP - 1, :, cs]], axis=0))
                    out_vm[r, cs] = (x_vm[r, cs].astype(f32) + s * gate).astype(bf16)
                    oc = OC if n == NR - 1 else (KD - 1,)
                    if nn in oc:
                        c0 = max([a + 1 for a in oc if a < nn], default=0)
                        cc = pl.ds(c0 * 128, (nn + 1 - c0) * 128)
                        pltpu.make_async_copy(out_vm.at[r, cc], out_hbm.at[r, cc], out_sem.at[0]).start()
        with scope("w_out"):
            pltpu.make_async_copy(out_vm, out_hbm, out_sem.at[0]).wait()

    def fn(A_x, A_k_cache, A_v_cache, A_wq, A_wo, B_x, B_w_r, B_w_gate, B_w_up, B_w_down):
        hbm = pl.BlockSpec(memory_space=pltpu.HBM)
        dma = pltpu.SemaphoreType.DMA
        out = pl.pallas_call(
            kernel,
            in_specs=[hbm] * 9,
            out_specs=hbm,
            out_shape=jax.ShapeDtypeStruct((S, D), bf16),
            scratch_shapes=[
                pltpu.VMEM((S, D), bf16), pltpu.VMEM((S, D), bf16),
                pltpu.VMEM((H, S, DH), bf16), pltpu.VMEM((H, S, DH), bf16), pltpu.VMEM((S, D), f32),
                pltpu.VMEM((NP, D, 256), bf16), pltpu.VMEM((NP, 256, D), bf16), pltpu.VMEM((3, F, D), bf16),
                pltpu.VMEM((2, 2, 2, S, DH), bf16), pltpu.VMEM((S, D), bf16), pltpu.VMEM((D,), bf16),
                pltpu.VMEM((3, 8, 128), f32), pltpu.VMEM((8, D), f32), pltpu.VMEM((8, D), f32),
                dma((2,)), dma((2,)), dma((1,)), dma((1,)),
            ],
            compiler_params=pltpu.CompilerParams(vmem_limit_bytes=110 * 2**20, flags=flags, disable_bounds_checks=nobc),
        )(A_x.reshape(S, D), A_k_cache.reshape(H, S, DH), A_v_cache.reshape(H, S, DH), A_wq, A_wo.reshape(NP, 256, D),
          B_w_r, B_w_gate.T, B_w_up.T, B_w_down)
        return out.reshape(1, S, D)
    return fn


@jax.jit
def pallas_recurrent_scan__mha_block_cached__moe_arch_mod__prompt_kernel(
    A_x, A_k_cache, A_v_cache, A_wq, A_wo, B_x, B_w_r, B_w_gate, B_w_up, B_w_down
):
    return _build()(A_x, A_k_cache, A_v_cache, A_wq, A_wo, B_x, B_w_r, B_w_gate, B_w_up, B_w_down)
```

```python
import jax
import jax.numpy as jnp
import numpy as np
from jax import lax
from jax.experimental import pallas as pl
from jax.experimental.pallas import tpu as pltpu

S, D, H, DH, F, C = 2048, 640, 32, 128, 1728, 8
KD = D // 128
NP = H // 2
TQ = 256
NR = S // TQ
NU = NR - 1
CK = 512
NC = S // CK
FB = 128
T0 = 128
XO = (0, 2, 4, 8, 16)
LN_DUE = (2, 3, 4, 5, 8)

f32, bf16, i32 = jnp.float32, jnp.bfloat16, jnp.int32
QSCALE = float(DH ** -0.5 * np.log2(np.e))
EPS = 1.0013580322265625e-05


def _fold(xs, op):
    r = xs[0]
    for a in xs[1:]:
        r = op(r, a)
    return r


def _cols(a, w=128):
    return [a[:, j * w:(j + 1) * w] for j in range(a.shape[1] // w)]


def _rows(a, w):
    return [a[j * w:(j + 1) * w, :] for j in range(a.shape[0] // w)]


def _round(a):
    return a.astype(bf16).astype(f32)


def _sigmoid(a):
    return pl.reciprocal(1.0 + jnp.exp(-a), approx=True)


def _dot(a, b):
    return lax.dot_general(a, b, (((1,), (0,)), ((), ())), preferred_element_type=f32)


def _dot_nt(a, b):
    return lax.dot_general(a, b, (((1,), (1,)), ((), ())), preferred_element_type=f32)


def _after(val, deps, zero):
    deps = [pltpu.bitcast(d, i32) for d in deps if d is not None]
    if not deps:
        return val
    return pltpu.bitcast(pltpu.bitcast(val, i32) | (_fold(deps, jnp.bitwise_or) & zero), val.dtype)


def _after_rows(lhs, deps, zero):
    if not deps:
        return lhs
    head = jnp.concatenate([_after(g, deps.get(n, []), zero) for n, g in enumerate(_rows(lhs[:, 0:128], 16))], axis=0)
    return head if lhs.shape[1] == 128 else jnp.concatenate([head, lhs[:, 128:]], axis=1)


def _token(key_bits):
    return (S - 1) - (key_bits & (S - 1))


def _token_group(tok):
    return pl.ds(pl.multiple_of((tok >> 4) << 4, 16), 16)


def _kernel(x_hbm, k_hbm, v_hbm, wq_hbm, wo_hbm, wr_hbm, wg_hbm, wu_hbm, wd_hbm, out_hbm,
            x_vm, xn_vm, q_vm, o_vm, s_vm, wq_vm, wo_vm, wf_vm, kv_vm, out_vm, wr_vm,
            key_vm, sel_vm, y_vm, x_sem, w_sem, kv_sem, io_sem):

    def x_copy(i):
        r = pl.ds(XO[i] * T0, (XO[i + 1] - XO[i]) * T0)
        return pltpu.make_async_copy(x_hbm.at[r, :], x_vm.at[r, :], x_sem.at[i % 2])

    def w_copies(part):
        sem = w_sem.at[part % 2]
        p0, p1 = ((0, 2), (2, 3), (3, NP))[part]
        cps = [pltpu.make_async_copy(wq_hbm.at[:, pl.ds(p * 256, 256)], wq_vm.at[p], sem) for p in range(p0, p1)]
        if part > 0:
            r = (pl.ds(0, 1), pl.ds(1, NP - 1))[part - 1]
            cps.append(pltpu.make_async_copy(wo_hbm.at[r], wo_vm.at[r], sem))
            r = (pl.ds(0, FB), pl.ds(FB, F - FB))[part - 1]
            cps += [pltpu.make_async_copy(w.at[r, :], wf_vm.at[a, r, :], sem)
                    for a, w in enumerate((wg_hbm, wu_hbm, wd_hbm))]
        return cps

    def kv_start(pair, slot):
        hs = pl.ds(pair * 2, 2)
        pltpu.make_async_copy(k_hbm.at[hs], kv_vm.at[slot, 0], kv_sem.at[0]).start()
        pltpu.make_async_copy(v_hbm.at[hs], kv_vm.at[slot, 1], kv_sem.at[0]).start()

    def kv_wait(slot):
        pltpu.make_async_copy(kv_vm.at[slot], kv_vm.at[slot], kv_sem.at[0]).wait()

    wr_copy = pltpu.make_async_copy(wr_hbm, wr_vm, io_sem.at[0])
    wr_copy.start()
    x_copy(0).start()
    for cp in w_copies(0):
        cp.start()

    def clear(n, carry):
        s_vm[pl.ds(pl.multiple_of(n * TQ, TQ), TQ), :] = jnp.zeros((TQ, D), f32)
        return carry

    lax.fori_loop(0, NR, clear, 0)
    y_vm[...] = jnp.zeros_like(y_vm)
    sel_vm[...] = jnp.zeros_like(sel_vm)
    wr_copy.wait()
    x_copy(0).wait()
    x_copy(1).start()
    wr = wr_vm[...].astype(f32).reshape(1, D)
    zero0 = lax.shift_right_logical(pltpu.bitcast(jnp.broadcast_to(wr[:, 0:128], (8, 128)), i32)[0, 0] & 1, 1)
    lane = lax.broadcasted_iota(i32, (8, 128), 1)
    sub = lax.broadcasted_iota(i32, (8, 128), 0)
    router = [jnp.zeros((8, 128), f32), jnp.zeros((8, 128), f32)]

    def layernorm(r0, n, start=None):
        r = pl.ds(r0, n)
        x = x_vm[r, :].astype(f32)
        if start is not None:
            xs = _cols(x)
            x = jnp.concatenate([_after(xs[0], [start], zero0)] + xs[1:], axis=1)
        mean = jnp.sum(x, axis=-1, keepdims=True) * (1.0 / D)
        yield mean
        shift = _round(mean)
        d = x - shift
        var = jnp.maximum(jnp.sum(d * d, axis=-1, keepdims=True) * (1.0 / D) - (mean - shift) * (mean - shift), 0.0)
        yield var
        inv = pl.reciprocal(_round(jnp.sqrt(_round(_round(var) + EPS))), approx=True)
        yield inv
        xn = d * inv
        xn_vm[r, :] = xn.astype(bf16)
        part = _fold(_cols(xn * wr), jnp.add)
        yield part
        score = jnp.broadcast_to(jnp.sum(part, axis=-1, keepdims=True), (n, 128))
        packed = []
        for a, sc in enumerate(_rows(score, 8)):
            g = r0 // 8 + a
            router[g // 128] = jnp.where(lane == g % 128, sc, router[g // 128])
            packed.append(router[g // 128])
        yield jnp.concatenate(packed, axis=0)

    for _ in layernorm(0, XO[1] * T0):
        pass
    for cp in w_copies(0):
        cp.wait()
    x_copy(2).start()
    due = {}
    prev = None
    assert LN_DUE[3] <= KD
    for n in range(S // T0):
        t = n + 1
        if XO[1] <= t < S // T0:
            if t in XO:
                x_copy(XO.index(t)).wait()
                if t == XO[1]:
                    x_copy(3).start()
                if t == XO[2]:
                    kv_start(0, 0)
                    for cp in w_copies(1):
                        cp.start()
                prev = None
            stages = layernorm(t * T0, T0, prev)
            for a in LN_DUE:
                due.setdefault(n * KD + a, []).append(stages)
        if n == S // T0 - 2:
            for cp in w_copies(2):
                cp.start()
        r = pl.ds(n * T0, T0)
        acc = None
        for k in range(KD):
            ks = slice(k * 128, (k + 1) * 128)
            vs = [_rows(jnp.broadcast_to(next(stages), (T0, 128)), 8) for stages in due.pop(n * KD + k, [])]
            deps = {a: [v[2 * a] for v in vs] for a in range(T0 // 16)} if vs else {}
            d = _dot(_after_rows(xn_vm[r, ks], deps, zero0),
                     jnp.concatenate([wq_vm[0, ks, :], wq_vm[1, ks, :]], axis=1))
            acc = d if acc is None else acc + d
            if k == 3:
                prev = d[:, 0:128]
        for c, qc in enumerate(_cols(acc * QSCALE)):
            q_vm[c, r, :] = qc.astype(bf16)
    assert not due
    for a in range(2):
        rb = _round(router[a])
        rb = jnp.where(rb == 0.0, 0.0, rb)
        bits = lax.shift_right_logical(pltpu.bitcast(rb, i32), 16)
        u = jnp.where(bits >= 0x8000, 0xFFFF - bits, bits + 0x8000)
        u = jnp.where(rb != rb, 0, u)
        key_vm[a] = pltpu.bitcast((1 << 29) + u * S + (S - 1 - (a * 1024 + lane * 8 + sub)), f32)
    for cp in w_copies(1):
        cp.wait()

    def step(g, carry):
        slot = g & 1
        kv_wait(slot)

        @pl.when(g == 1)
        def _():
            for cp in w_copies(2):
                cp.wait()
            row16 = lax.broadcasted_iota(i32, (16, D), 0)
            kbits = pltpu.bitcast(key_vm[2], i32)
            xsel = jnp.zeros((16, D), f32)
            for c in range(C):
                tok = _token(kbits[c, 0])
                grp = xn_vm[_token_group(tok), :].astype(f32)
                rowv = jnp.sum(jnp.where(row16 == (tok & 15), grp, 0.0), axis=0, keepdims=True)
                xsel = jnp.where(row16 == c, rowv, xsel)
            sel_vm[...] = xsel[0:C, :]

        zero = lax.shift_right_logical(g, 8)

        st = dict(k0=key_vm[0], k1=key_vm[1], keys=jnp.zeros((8, 128), f32))
        f0 = pl.multiple_of(jnp.clip((g - 1) * FB, 0, F - FB), 64)

        def pick(c):
            k0, k1 = st["k0"], st["k1"]
            mx = jnp.max(jnp.max(jnp.maximum(k0, k1), axis=1, keepdims=True), axis=0, keepdims=True)
            st["k0"] = jnp.where(k0 == mx, 0.0, k0)
            st["k1"] = jnp.where(k1 == mx, 0.0, k1)
            st["keys"] = jnp.where(sub == c, mx, st["keys"])
            if c == C - 1:
                key_vm[2] = st["keys"]
            return {0: [st["keys"]]}

        def gate_up(k):
            ks = slice(k * 256, min((k + 1) * 256, D))
            w = jnp.concatenate([wf_vm[0, pl.ds(f0, FB), ks], wf_vm[1, pl.ds(f0, FB), ks]], axis=0)
            d = _dot_nt(sel_vm[:, ks].astype(bf16), w)
            st["gu"] = d if k == 0 else st["gu"] + d
            return {}

        def hidden():
            unit_id = f0 + lax.broadcasted_iota(i32, (C, FB), 1)
            gate, up = _cols(st["gu"], FB)
            fresh = unit_id >= jnp.where(g == 0, F, (g - 1) * FB)
            st["hid"] = _round(jnp.where(fresh, gate * _sigmoid(gate) * up, 0.0))
            return {0: [st["hid"]]}

        def down(n):
            cs = slice(n * 512, min((n + 1) * 512, D))
            y_vm[:, cs] += _dot(st["hid"].astype(bf16), wf_vm[2, pl.ds(f0, FB), cs])
            return {}

        tasks = {}
        for c in range(C):
            tasks.setdefault((1 + c // 4, 0), []).append(lambda c=c: pick(c))
        for k in range(3):
            tasks[4, k] = [lambda k=k: gate_up(k)]
        tasks[5, 0] = [hidden]
        for k in range(2):
            tasks[6, k] = [lambda k=k: down(k)]

        def routed(j, a):
            return ([{}] + [f() for f in tasks.get((j, a), [])])[-1]

        def unit(j):
            u = g * NU + j
            return u >> 3, pl.multiple_of((u & 7) * TQ, TQ)

        def q_unit(j):
            p, r0 = unit(j)
            r = pl.ds(r0, TQ)
            ds = [_dot(_after_rows(xn_vm[r, 0:512], routed(j, a), zero), wq_vm[p + 2, 0:512, a * 128:(a + 1) * 128])
                  for a in range(2)]
            rest = [_dot(_after_rows(xn_vm[pl.ds(r0 + a * 128, 128), 512:D], routed(j, 2 + a), zero),
                         wq_vm[p + 2, 512:D, :]) for a in range(2)]
            q = (jnp.concatenate(ds, axis=1) + jnp.concatenate(rest, axis=0)) * QSCALE
            for c, qc in enumerate(_cols(q)):
                q_vm[2 * p + 4 + c, r, :] = qc.astype(bf16)
            return ds[1]

        def o_unit(j):
            p, r0 = unit(j)
            o = jnp.concatenate([o_vm[2 * p + c, pl.ds(r0, TQ), :] for c in range(2)], axis=1)
            left = _dot(o[:, 0:128], wo_vm[p, 0:128, 0:512]) + _dot(o[:, 128:256], wo_vm[p, 128:256, 0:512])
            right = jnp.concatenate([_dot(oa, wo_vm[p, :, 512:D]) for oa in _rows(o, 128)], axis=0)
            s_vm[pl.ds(r0, TQ), :] += jnp.concatenate([left, right], axis=1)
            return right

        pending = []

        def store_o(dep):
            t, o = pending.pop()
            deps = {} if dep is None else {a: [d] for a, d in enumerate(_rows(dep, 8)[::2])}
            o_vm[g * 2 + t["h"], t["r"], :] = _after_rows(o, deps, zero)

        def scores(n):
            t = dict(h=n // NR, r=pl.ds(n % NR * TQ, TQ), s=[], sum=None)
            q = q_vm[g * 2 + t["h"], t["r"], :]
            t["unit"] = q_unit(n) if n < NU else None
            for c in range(NC):
                s = _cols(_dot_nt(q, kv_vm[slot, 0, t["h"], c * CK:(c + 1) * CK, :]))
                mc = jnp.maximum(jnp.maximum(s[0], s[1]), jnp.maximum(s[2], s[3]))
                m = mc if c == 0 else jnp.maximum(m, mc)
                t["s"].append(s)
                if c == 1 and pending:
                    store_o(s[0])
            t["max"] = jnp.broadcast_to(jnp.max(m, axis=-1, keepdims=True), (TQ, 128))
            return t

        def probs(t, c, dep):
            t["max"] = _after(t["max"], [dep, t["sum"]], zero)
            ps = [jnp.exp2(s - t["max"]) for s in t["s"][c]]
            part = _fold(ps, jnp.add)
            t["sum"] = part if c == 0 else t["sum"] + part
            return jnp.concatenate(ps, axis=1).astype(bf16)

        cur = scores(0)
        kv_start(jnp.minimum(g + 1, NP - 1), 1 - slot)
        for n in range(2 * NR):
            nxt = scores(n + 1) if n + 1 < 2 * NR else None
            if n == 0:
                last = nxt["unit"]
            for c in range(NC):
                last = _dot(probs(cur, c, last), kv_vm[slot, 1, cur["h"], c * CK:(c + 1) * CK, :])
                acc = last if c == 0 else acc + last
            l = jnp.sum(cur["sum"], axis=-1, keepdims=True)
            rl = pl.reciprocal(l, approx=True)
            last = acc * (rl * (2.0 - l * rl))
            done = o_unit(n - NR - 1) if n > NR else None
            pending.append((cur, last.astype(bf16)))
            if n <= NR or n + 2 >= 2 * NR:
                store_o(done)
            cur = nxt
        assert not pending
        return carry

    lax.fori_loop(0, NP, step, 0)
    kv_wait(NP & 1)

    kbits = pltpu.bitcast(key_vm[2], i32)
    u = lax.shift_right_logical(kbits, 11) & 0xFFFF
    rsel = pltpu.bitcast(jnp.where(u >= 0x8000, u - 0x8000, 0xFFFF - u) << 16, f32)
    bsel = sel_vm[...] + y_vm[...] * jnp.tile(_sigmoid(rsel), (1, KD))
    row16 = lax.broadcasted_iota(i32, (16, D), 0)
    for c in range(C):
        tok = _token(kbits[c, 0])
        grp = xn_vm[_token_group(tok), :].astype(f32)
        xn_vm[_token_group(tok), :] = jnp.where(row16 == (tok & 15), bsel[c:c + 1, :], grp).astype(bf16)

    for n in range(NR):
        r = pl.ds(n * TQ, TQ)
        sent = 0
        for k in range(KD):
            cs = slice(k * 128, (k + 1) * 128)
            b = xn_vm[r, cs].astype(f32)
            gate = b * _sigmoid(b)
            o = jnp.concatenate([o_vm[H - 4 + a, r, :] for a in range(4)], axis=1)
            if n > 0:
                o = _after_rows(o, {a: [d] for a, d in enumerate(_rows(gate, 8)[1::2])}, zero0)
            s = s_vm[r, cs] + _dot(o, jnp.concatenate([wo_vm[NP - 2, :, cs], wo_vm[NP - 1, :, cs]], axis=0))
            out_vm[r, cs] = (x_vm[r, cs].astype(f32) + s * gate).astype(bf16)
            if k == KD - 1 or (n == NR - 1 and k > 0):
                cc = pl.ds(sent * 128, (k + 1 - sent) * 128)
                pltpu.make_async_copy(out_vm.at[r, cc], out_hbm.at[r, cc], io_sem.at[0]).start()
                sent = k + 1
    pltpu.make_async_copy(out_vm, out_hbm, io_sem.at[0]).wait()


@jax.jit
def pallas_recurrent_scan__mha_block_cached__moe_arch_mod__prompt_kernel(
    A_x: jax.Array,
    A_k_cache: jax.Array,
    A_v_cache: jax.Array,
    A_wq: jax.Array,
    A_wo: jax.Array,
    B_x: jax.Array,
    B_w_r: jax.Array,
    B_w_gate: jax.Array,
    B_w_up: jax.Array,
    B_w_down: jax.Array,
):
    del B_x
    hbm = pl.BlockSpec(memory_space=pltpu.HBM)
    dma = pltpu.SemaphoreType.DMA
    out = pl.pallas_call(
        _kernel,
        in_specs=[hbm] * 9,
        out_specs=hbm,
        out_shape=jax.ShapeDtypeStruct((S, D), bf16),
        scratch_shapes=[
            pltpu.VMEM((S, D), bf16),
            pltpu.VMEM((S, D), bf16),
            pltpu.VMEM((H, S, DH), bf16),
            pltpu.VMEM((H, S, DH), bf16),
            pltpu.VMEM((S, D), f32),
            pltpu.VMEM((NP, D, 256), bf16),
            pltpu.VMEM((NP, 256, D), bf16),
            pltpu.VMEM((3, F, D), bf16),
            pltpu.VMEM((2, 2, 2, S, DH), bf16),
            pltpu.VMEM((S, D), bf16),
            pltpu.VMEM((D,), bf16),
            pltpu.VMEM((3, 8, 128), f32),
            pltpu.VMEM((C, D), f32),
            pltpu.VMEM((C, D), f32),
            dma((2,)), dma((2,)), dma((1,)), dma((1,)),
        ],
        compiler_params=pltpu.CompilerParams(vmem_limit_bytes=110 * 2**20),
    )(A_x.reshape(S, D), A_k_cache.reshape(H, S, DH), A_v_cache.reshape(H, S, DH), A_wq,
      A_wo.reshape(NP, 256, D), B_w_r, B_w_gate.T, B_w_up.T, B_w_down)
    return out.reshape(1, S, D)
```

```python
import jax
import jax.numpy as jnp
import numpy as np
from jax import lax
from jax.experimental import pallas as pl
from jax.experimental.pallas import tpu as pltpu

S, D, H, DH, F, C = 2048, 640, 32, 128, 1728, 8
KD = D // 128
NP = H // 2
TQ = 256
NR = S // TQ
NU = NR - 1
CK = 512
NC = S // CK
FB = 128
T0 = 128
XO = (0, 2, 4, 8, 16)
LN_DUE = (2, 3, 4, 5, 8)

f32, bf16, i32 = jnp.float32, jnp.bfloat16, jnp.int32
QSCALE = float(DH ** -0.5 * np.log2(np.e))
EPS = 1.0013580322265625e-05


def _fold(xs, op):
    r = xs[0]
    for a in xs[1:]:
        r = op(r, a)
    return r


def _cols(a, w=128):
    return [a[:, j * w:(j + 1) * w] for j in range(a.shape[1] // w)]


def _rows(a, w):
    return [a[j * w:(j + 1) * w, :] for j in range(a.shape[0] // w)]


def _round(a):
    return a.astype(bf16).astype(f32)


def _sigmoid(a):
    return pl.reciprocal(1.0 + jnp.exp(-a), approx=True)


def _dot(a, b):
    return lax.dot_general(a, b, (((1,), (0,)), ((), ())), preferred_element_type=f32)


def _dot_nt(a, b):
    return lax.dot_general(a, b, (((1,), (1,)), ((), ())), preferred_element_type=f32)


def _after(val, deps, zero):
    deps = [pltpu.bitcast(d, i32) for d in deps if d is not None]
    if not deps:
        return val
    return pltpu.bitcast(pltpu.bitcast(val, i32) | (_fold(deps, jnp.bitwise_or) & zero), val.dtype)


def _after_rows(lhs, deps, zero):
    if not deps:
        return lhs
    head = jnp.concatenate([_after(g, deps.get(n, []), zero) for n, g in enumerate(_rows(lhs[:, 0:128], 16))], axis=0)
    return head if lhs.shape[1] == 128 else jnp.concatenate([head, lhs[:, 128:]], axis=1)


def _token(key_bits):
    return (S - 1) - (key_bits & (S - 1))


def _token_group(tok):
    return pl.ds(pl.multiple_of((tok >> 4) << 4, 16), 16)


def _kernel(x_hbm, k_hbm, v_hbm, wq_hbm, wo_hbm, wr_hbm, wg_hbm, wu_hbm, wd_hbm, out_hbm,
            x_vm, xn_vm, q_vm, o_vm, s_vm, wq0_vm, wq_vm, wo_vm, wf_vm, kv_vm, out_vm, wr_vm,
            key_vm, sel_vm, y_vm, x_sem, w_sem, kv_sem, io_sem):

    def x_copy(i):
        r = pl.ds(XO[i] * T0, (XO[i + 1] - XO[i]) * T0)
        return pltpu.make_async_copy(x_hbm.at[r, :], x_vm.at[r, :], x_sem.at[i % 2])

    def w_copies(part):
        sem = w_sem.at[part % 2]
        if part == 0:
            return [pltpu.make_async_copy(wq_hbm.at[:, pl.ds(0, 512)], wq0_vm, sem)]
        cps = [pltpu.make_async_copy(wq_hbm.at[:, pl.ds((p + 2) * 256, 256)], wq_vm.at[p], sem)
               for p in (range(0, 1), range(1, NP - 2))[part - 1]]
        r = (pl.ds(0, 1), pl.ds(1, NP - 1))[part - 1]
        cps.append(pltpu.make_async_copy(wo_hbm.at[r], wo_vm.at[r], sem))
        r = (pl.ds(0, FB), pl.ds(FB, F - FB))[part - 1]
        cps += [pltpu.make_async_copy(w.at[r, :], wf_vm.at[a, r, :], sem)
                for a, w in enumerate((wg_hbm, wu_hbm, wd_hbm))]
        return cps

    def kv_start(pair, slot):
        hs = pl.ds(pair * 2, 2)
        pltpu.make_async_copy(k_hbm.at[hs], kv_vm.at[slot, 0], kv_sem.at[0]).start()
        pltpu.make_async_copy(v_hbm.at[hs], kv_vm.at[slot, 1], kv_sem.at[0]).start()

    def kv_wait(slot):
        pltpu.make_async_copy(kv_vm.at[slot], kv_vm.at[slot], kv_sem.at[0]).wait()

    wr_copy = pltpu.make_async_copy(wr_hbm, wr_vm, io_sem.at[0])
    wr_copy.start()
    x_copy(0).start()
    for cp in w_copies(0):
        cp.start()

    def clear(n, carry):
        s_vm[pl.ds(pl.multiple_of(n * TQ, TQ), TQ), :] = jnp.zeros((TQ, D), f32)
        return carry

    lax.fori_loop(0, NR, clear, 0)
    y_vm[...] = jnp.zeros_like(y_vm)
    sel_vm[...] = jnp.zeros_like(sel_vm)
    wr_copy.wait()
    x_copy(0).wait()
    x_copy(1).start()
    wr = wr_vm[...].astype(f32).reshape(1, D)
    zero0 = lax.shift_right_logical(pltpu.bitcast(jnp.broadcast_to(wr[:, 0:128], (8, 128)), i32)[0, 0] & 1, 1)
    lane = lax.broadcasted_iota(i32, (8, 128), 1)
    sub = lax.broadcasted_iota(i32, (8, 128), 0)
    router = [jnp.zeros((8, 128), f32), jnp.zeros((8, 128), f32)]

    def layernorm(r0, n, start=None):
        r = pl.ds(r0, n)
        x = x_vm[r, :].astype(f32)
        if start is not None:
            xs = _cols(x)
            x = jnp.concatenate([_after(xs[0], [start], zero0)] + xs[1:], axis=1)
        mean = jnp.sum(x, axis=-1, keepdims=True) * (1.0 / D)
        yield mean
        shift = _round(mean)
        d = x - shift
        var = jnp.maximum(jnp.sum(d * d, axis=-1, keepdims=True) * (1.0 / D) - (mean - shift) * (mean - shift), 0.0)
        yield var
        inv = pl.reciprocal(_round(jnp.sqrt(_round(_round(var) + EPS))), approx=True)
        yield inv
        xn = d * inv
        xn_vm[r, :] = xn.astype(bf16)
        part = _fold(_cols(xn * wr), jnp.add)
        yield part
        score = jnp.broadcast_to(jnp.sum(part, axis=-1, keepdims=True), (n, 128))
        packed = []
        for a, sc in enumerate(_rows(score, 8)):
            g = r0 // 8 + a
            router[g // 128] = jnp.where(lane == g % 128, sc, router[g // 128])
            packed.append(router[g // 128])
        yield jnp.concatenate(packed, axis=0)

    for _ in layernorm(0, XO[1] * T0):
        pass
    for cp in w_copies(0):
        cp.wait()
    x_copy(2).start()
    due = {}
    prev = None
    assert LN_DUE[3] <= KD
    for n in range(S // T0):
        t = n + 1
        if XO[1] <= t < S // T0:
            if t in XO:
                x_copy(XO.index(t)).wait()
                if t == XO[1]:
                    x_copy(3).start()
                if t == XO[2]:
                    kv_start(0, 0)
                    for cp in w_copies(1):
                        cp.start()
                prev = None
            stages = layernorm(t * T0, T0, prev)
            for a in LN_DUE:
                due.setdefault(n * KD + a, []).append(stages)
        if n == S // T0 - 2:
            for cp in w_copies(2):
                cp.start()
        r = pl.ds(n * T0, T0)
        acc = None
        for k in range(KD):
            ks = slice(k * 128, (k + 1) * 128)
            vs = [_rows(jnp.broadcast_to(next(stages), (T0, 128)), 8) for stages in due.pop(n * KD + k, [])]
            deps = {a: [v[2 * a] for v in vs] for a in range(T0 // 16)} if vs else {}
            d = _dot(_after_rows(xn_vm[r, ks], deps, zero0), wq0_vm[ks, :])
            acc = d if acc is None else acc + d
            if k == 3:
                prev = d[:, 0:128]
        for c, qc in enumerate(_cols(acc * QSCALE)):
            q_vm[c, r, :] = qc.astype(bf16)
    assert not due
    for a in range(2):
        rb = _round(router[a])
        rb = jnp.where(rb == 0.0, 0.0, rb)
        bits = lax.shift_right_logical(pltpu.bitcast(rb, i32), 16)
        u = jnp.where(bits >= 0x8000, 0xFFFF - bits, bits + 0x8000)
        u = jnp.where(rb != rb, 0, u)
        key_vm[a] = pltpu.bitcast((1 << 29) + u * S + (S - 1 - (a * 1024 + lane * 8 + sub)), f32)
    for cp in w_copies(1):
        cp.wait()

    def step(g, carry):
        slot = g & 1
        kv_wait(slot)

        @pl.when(g == 1)
        def _():
            for cp in w_copies(2):
                cp.wait()
            row16 = lax.broadcasted_iota(i32, (16, D), 0)
            kbits = pltpu.bitcast(key_vm[2], i32)
            xsel = jnp.zeros((16, D), f32)
            for c in range(C):
                tok = _token(kbits[c, 0])
                grp = xn_vm[_token_group(tok), :].astype(f32)
                rowv = jnp.sum(jnp.where(row16 == (tok & 15), grp, 0.0), axis=0, keepdims=True)
                xsel = jnp.where(row16 == c, rowv, xsel)
            sel_vm[...] = xsel[0:C, :]

        zero = lax.shift_right_logical(g, 8)

        st = dict(k0=key_vm[0], k1=key_vm[1], keys=jnp.zeros((8, 128), f32))
        f0 = pl.multiple_of(jnp.clip((g - 1) * FB, 0, F - FB), 64)

        def pick(c):
            k0, k1 = st["k0"], st["k1"]
            mx = jnp.max(jnp.max(jnp.maximum(k0, k1), axis=1, keepdims=True), axis=0, keepdims=True)
            st["k0"] = jnp.where(k0 == mx, 0.0, k0)
            st["k1"] = jnp.where(k1 == mx, 0.0, k1)
            st["keys"] = jnp.where(sub == c, mx, st["keys"])
            if c == C - 1:
                key_vm[2] = st["keys"]
            return {0: [st["keys"]]}

        def gate_up(k):
            ks = slice(k * 256, min((k + 1) * 256, D))
            w = jnp.concatenate([wf_vm[0, pl.ds(f0, FB), ks], wf_vm[1, pl.ds(f0, FB), ks]], axis=0)
            d = _dot_nt(sel_vm[:, ks].astype(bf16), w)
            st["gu"] = d if k == 0 else st["gu"] + d
            return {}

        def hidden():
            unit_id = f0 + lax.broadcasted_iota(i32, (C, FB), 1)
            gate, up = _cols(st["gu"], FB)
            fresh = unit_id >= jnp.where(g == 0, F, (g - 1) * FB)
            st["hid"] = _round(jnp.where(fresh, gate * _sigmoid(gate) * up, 0.0))
            return {0: [st["hid"]]}

        def down(n):
            cs = slice(n * 512, min((n + 1) * 512, D))
            y_vm[:, cs] += _dot(st["hid"].astype(bf16), wf_vm[2, pl.ds(f0, FB), cs])
            return {}

        tasks = {}
        for c in range(C):
            tasks.setdefault((1 + c // 4, 0), []).append(lambda c=c: pick(c))
        for k in range(3):
            tasks[4, k] = [lambda k=k: gate_up(k)]
        tasks[5, 0] = [hidden]
        for k in range(2):
            tasks[6, k] = [lambda k=k: down(k)]

        def routed(j, a):
            return ([{}] + [f() for f in tasks.get((j, a), [])])[-1]

        def unit(j):
            u = g * NU + j
            return u >> 3, pl.multiple_of((u & 7) * TQ, TQ)

        def q_unit(j):
            p, r0 = unit(j)
            r = pl.ds(r0, TQ)
            ds = [_dot(_after_rows(xn_vm[r, 0:512], routed(j, a), zero), wq_vm[p, 0:512, a * 128:(a + 1) * 128])
                  for a in range(2)]
            rest = [_dot(_after_rows(xn_vm[pl.ds(r0 + a * 128, 128), 512:D], routed(j, 2 + a), zero),
                         wq_vm[p, 512:D, :]) for a in range(2)]
            q = (jnp.concatenate(ds, axis=1) + jnp.concatenate(rest, axis=0)) * QSCALE
            for c, qc in enumerate(_cols(q)):
                q_vm[2 * p + 4 + c, r, :] = qc.astype(bf16)
            return ds[1]

        def o_unit(j):
            p, r0 = unit(j)
            o = jnp.concatenate([o_vm[2 * p + c, pl.ds(r0, TQ), :] for c in range(2)], axis=1)
            left = _dot(o[:, 0:128], wo_vm[p, 0:128, 0:512]) + _dot(o[:, 128:256], wo_vm[p, 128:256, 0:512])
            right = jnp.concatenate([_dot(oa, wo_vm[p, :, 512:D]) for oa in _rows(o, 128)], axis=0)
            s_vm[pl.ds(r0, TQ), :] += jnp.concatenate([left, right], axis=1)
            return right

        pending = []

        def store_o(dep):
            t, o = pending.pop()
            deps = {} if dep is None else {a: [d] for a, d in enumerate(_rows(dep, 8)[::2])}
            o_vm[g * 2 + t["h"], t["r"], :] = _after_rows(o, deps, zero)

        def scores(n):
            t = dict(h=n // NR, r=pl.ds(n % NR * TQ, TQ), s=[], sum=None)
            q = q_vm[g * 2 + t["h"], t["r"], :]
            t["unit"] = q_unit(n) if n < NU else None
            for c in range(NC):
                s = _cols(_dot_nt(q, kv_vm[slot, 0, t["h"], c * CK:(c + 1) * CK, :]))
                mc = jnp.maximum(jnp.maximum(s[0], s[1]), jnp.maximum(s[2], s[3]))
                m = mc if c == 0 else jnp.maximum(m, mc)
                t["s"].append(s)
                if c == 1 and pending:
                    store_o(s[0])
            t["max"] = jnp.broadcast_to(jnp.max(m, axis=-1, keepdims=True), (TQ, 128))
            return t

        def probs(t, c, dep):
            t["max"] = _after(t["max"], [dep, t["sum"]], zero)
            ps = [jnp.exp2(s - t["max"]) for s in t["s"][c]]
            part = _fold(ps, jnp.add)
            t["sum"] = part if c == 0 else t["sum"] + part
            return jnp.concatenate(ps, axis=1).astype(bf16)

        cur = scores(0)
        kv_start(jnp.minimum(g + 1, NP - 1), 1 - slot)
        for n in range(2 * NR):
            nxt = scores(n + 1) if n + 1 < 2 * NR else None
            if n == 0:
                last = nxt["unit"]
            for c in range(NC):
                last = _dot(probs(cur, c, last), kv_vm[slot, 1, cur["h"], c * CK:(c + 1) * CK, :])
                acc = last if c == 0 else acc + last
            l = jnp.sum(cur["sum"], axis=-1, keepdims=True)
            rl = pl.reciprocal(l, approx=True)
            last = acc * (rl * (2.0 - l * rl))
            done = o_unit(n - NR - 1) if n > NR else None
            pending.append((cur, last.astype(bf16)))
            if n <= NR or n + 2 >= 2 * NR:
                store_o(done)
            cur = nxt
        assert not pending
        return carry

    lax.fori_loop(0, NP, step, 0)
    kv_wait(NP & 1)

    kbits = pltpu.bitcast(key_vm[2], i32)
    u = lax.shift_right_logical(kbits, 11) & 0xFFFF
    rsel = pltpu.bitcast(jnp.where(u >= 0x8000, u - 0x8000, 0xFFFF - u) << 16, f32)
    bsel = sel_vm[...] + y_vm[...] * jnp.tile(_sigmoid(rsel), (1, KD))
    row16 = lax.broadcasted_iota(i32, (16, D), 0)
    for c in range(C):
        tok = _token(kbits[c, 0])
        grp = xn_vm[_token_group(tok), :].astype(f32)
        xn_vm[_token_group(tok), :] = jnp.where(row16 == (tok & 15), bsel[c:c + 1, :], grp).astype(bf16)

    for n in range(NR):
        r = pl.ds(n * TQ, TQ)
        sent = 0
        for k in range(KD):
            cs = slice(k * 128, (k + 1) * 128)
            b = xn_vm[r, cs].astype(f32)
            gate = b * _sigmoid(b)
            o = jnp.concatenate([o_vm[H - 4 + a, r, :] for a in range(4)], axis=1)
            if n > 0:
                o = _after_rows(o, {a: [d] for a, d in enumerate(_rows(gate, 8)[1::2])}, zero0)
            s = s_vm[r, cs] + _dot(o, jnp.concatenate([wo_vm[NP - 2, :, cs], wo_vm[NP - 1, :, cs]], axis=0))
            out_vm[r, cs] = (x_vm[r, cs].astype(f32) + s * gate).astype(bf16)
            if k == KD - 1 or (n == NR - 1 and k > 0):
                cc = pl.ds(sent * 128, (k + 1 - sent) * 128)
                pltpu.make_async_copy(out_vm.at[r, cc], out_hbm.at[r, cc], io_sem.at[0]).start()
                sent = k + 1
    pltpu.make_async_copy(out_vm, out_hbm, io_sem.at[0]).wait()


@jax.jit
def pallas_recurrent_scan__mha_block_cached__moe_arch_mod__prompt_kernel(
    A_x: jax.Array,
    A_k_cache: jax.Array,
    A_v_cache: jax.Array,
    A_wq: jax.Array,
    A_wo: jax.Array,
    B_x: jax.Array,
    B_w_r: jax.Array,
    B_w_gate: jax.Array,
    B_w_up: jax.Array,
    B_w_down: jax.Array,
):
    del B_x
    hbm = pl.BlockSpec(memory_space=pltpu.HBM)
    dma = pltpu.SemaphoreType.DMA
    out = pl.pallas_call(
        _kernel,
        in_specs=[hbm] * 9,
        out_specs=hbm,
        out_shape=jax.ShapeDtypeStruct((S, D), bf16),
        scratch_shapes=[
            pltpu.VMEM((S, D), bf16),
            pltpu.VMEM((S, D), bf16),
            pltpu.VMEM((H, S, DH), bf16),
            pltpu.VMEM((H, S, DH), bf16),
            pltpu.VMEM((S, D), f32),
            pltpu.VMEM((D, 512), bf16),
            pltpu.VMEM((NP - 2, D, 256), bf16),
            pltpu.VMEM((NP, 256, D), bf16),
            pltpu.VMEM((3, F, D), bf16),
            pltpu.VMEM((2, 2, 2, S, DH), bf16),
            pltpu.VMEM((S, D), bf16),
            pltpu.VMEM((D,), bf16),
            pltpu.VMEM((3, 8, 128), f32),
            pltpu.VMEM((C, D), f32),
            pltpu.VMEM((C, D), f32),
            dma((2,)), dma((2,)), dma((1,)), dma((1,)),
        ],
        compiler_params=pltpu.CompilerParams(vmem_limit_bytes=110 * 2**20),
    )(A_x.reshape(S, D), A_k_cache.reshape(H, S, DH), A_v_cache.reshape(H, S, DH), A_wq,
      A_wo.reshape(NP, 256, D), B_w_r, B_w_gate.T, B_w_up.T, B_w_down)
    return out.reshape(1, S, D)
```

```python
import jax
import jax.numpy as jnp
import numpy as np
from jax import lax
from jax.experimental import pallas as pl
from jax.experimental.pallas import tpu as pltpu

S, D, H, DH, F, C = 2048, 640, 32, 128, 1728, 8
KD = D // 128
NP = H // 2
TQ = 256
NR = S // TQ
NU = NR - 1
CK = 512
NC = S // CK
FB = 128
T0 = 128
XO = (0, 2, 4, 8, 16)
LN_DUE = (2, 3, 4, 5, 8)

f32, bf16, i32 = jnp.float32, jnp.bfloat16, jnp.int32
QSCALE = float(DH ** -0.5 * np.log2(np.e))
EPS = 1.0013580322265625e-05


def _fold(xs, op):
    r = xs[0]
    for a in xs[1:]:
        r = op(r, a)
    return r


def _cols(a, w=128):
    return [a[:, j * w:(j + 1) * w] for j in range(a.shape[1] // w)]


def _rows(a, w):
    return [a[j * w:(j + 1) * w, :] for j in range(a.shape[0] // w)]


def _round(a):
    return a.astype(bf16).astype(f32)


def _sigmoid(a):
    return pl.reciprocal(1.0 + jnp.exp(-a), approx=True)


def _dot(a, b):
    return lax.dot_general(a, b, (((1,), (0,)), ((), ())), preferred_element_type=f32)


def _dot_nt(a, b):
    return lax.dot_general(a, b, (((1,), (1,)), ((), ())), preferred_element_type=f32)


def _after(val, deps, zero):
    deps = [pltpu.bitcast(d, i32) for d in deps if d is not None]
    if not deps:
        return val
    return pltpu.bitcast(pltpu.bitcast(val, i32) | (_fold(deps, jnp.bitwise_or) & zero), val.dtype)


def _after_rows(lhs, deps, zero):
    if not deps:
        return lhs
    head = jnp.concatenate([_after(g, deps.get(n, []), zero) for n, g in enumerate(_rows(lhs[:, 0:128], 16))], axis=0)
    return head if lhs.shape[1] == 128 else jnp.concatenate([head, lhs[:, 128:]], axis=1)


def _token(key_bits):
    return (S - 1) - (key_bits & (S - 1))


def _token_group(tok):
    return pl.ds(pl.multiple_of((tok >> 4) << 4, 16), 16)


def _kernel(x_hbm, k_hbm, v_hbm, wq_hbm, wo_hbm, wr_hbm, wg_hbm, wu_hbm, wd_hbm, out_hbm,
            x_vm, xn_vm, q_vm, o_vm, s_vm, wq0_vm, wq_vm, wo_vm, wf_vm, kv_vm, out_vm, wr_vm,
            key_vm, sel_vm, y_vm, x_sem, w_sem, kv_sem, io_sem):

    def x_copy(i):
        r = pl.ds(XO[i] * T0, (XO[i + 1] - XO[i]) * T0)
        return pltpu.make_async_copy(x_hbm.at[r, :], x_vm.at[r, :], x_sem.at[i % 2])

    def w_copies(part):
        sem = w_sem.at[part % 2]
        if part == 0:
            return [pltpu.make_async_copy(wq_hbm.at[:, pl.ds(0, 512)], wq0_vm, sem)]
        cps = [pltpu.make_async_copy(wq_hbm.at[:, pl.ds((p + 2) * 256, 256)], wq_vm.at[p], sem)
               for p in (range(0, 1), range(1, NP - 2))[part - 1]]
        r = (pl.ds(0, 1), pl.ds(1, NP - 1))[part - 1]
        cps.append(pltpu.make_async_copy(wo_hbm.at[r], wo_vm.at[r], sem))
        r = (pl.ds(0, FB), pl.ds(FB, F - FB))[part - 1]
        cps += [pltpu.make_async_copy(w.at[r, :], wf_vm.at[a, r, :], sem)
                for a, w in enumerate((wg_hbm, wu_hbm, wd_hbm))]
        return cps

    def kv_start(pair, slot):
        hs = pl.ds(pair * 2, 2)
        pltpu.make_async_copy(k_hbm.at[hs], kv_vm.at[slot, 0], kv_sem.at[0]).start()
        pltpu.make_async_copy(v_hbm.at[hs], kv_vm.at[slot, 1], kv_sem.at[0]).start()

    def kv_wait(slot):
        pltpu.make_async_copy(kv_vm.at[slot], kv_vm.at[slot], kv_sem.at[0]).wait()

    wr_copy = pltpu.make_async_copy(wr_hbm, wr_vm, io_sem.at[0])
    wr_copy.start()
    x_copy(0).start()
    for cp in w_copies(0):
        cp.start()

    def clear(n, carry):
        s_vm[pl.ds(pl.multiple_of(n * TQ, TQ), TQ), :] = jnp.zeros((TQ, D), f32)
        return carry

    lax.fori_loop(0, NR, clear, 0)
    y_vm[...] = jnp.zeros_like(y_vm)
    sel_vm[...] = jnp.zeros_like(sel_vm)
    wr_copy.wait()
    x_copy(0).wait()
    x_copy(1).start()
    wr = wr_vm[...].astype(f32).reshape(1, D)
    zero0 = lax.shift_right_logical(pltpu.bitcast(jnp.broadcast_to(wr[:, 0:128], (8, 128)), i32)[0, 0] & 1, 1)
    lane = lax.broadcasted_iota(i32, (8, 128), 1)
    sub = lax.broadcasted_iota(i32, (8, 128), 0)
    router = [jnp.zeros((8, 128), f32), jnp.zeros((8, 128), f32)]

    def layernorm(r0, n, start=None):
        r = pl.ds(r0, n)
        x = x_vm[r, :].astype(f32)
        if start is not None:
            xs = _cols(x)
            x = jnp.concatenate([_after(xs[0], [start], zero0)] + xs[1:], axis=1)
        mean = jnp.sum(x, axis=-1, keepdims=True) * (1.0 / D)
        yield mean
        shift = _round(mean)
        d = x - shift
        var = jnp.maximum(jnp.sum(d * d, axis=-1, keepdims=True) * (1.0 / D) - (mean - shift) * (mean - shift), 0.0)
        yield var
        inv = pl.reciprocal(_round(jnp.sqrt(_round(_round(var) + EPS))), approx=True)
        yield inv
        xn = d * inv
        xn_vm[r, :] = xn.astype(bf16)
        part = _fold(_cols(xn * wr), jnp.add)
        yield part
        score = jnp.broadcast_to(jnp.sum(part, axis=-1, keepdims=True), (n, 128))
        packed = []
        for a, sc in enumerate(_rows(score, 8)):
            g = r0 // 8 + a
            router[g // 128] = jnp.where(lane == g % 128, sc, router[g // 128])
            packed.append(router[g // 128])
        yield jnp.concatenate(packed, axis=0)

    for _ in layernorm(0, XO[1] * T0):
        pass
    for cp in w_copies(0):
        cp.wait()
    x_copy(2).start()
    due = {}
    prev = None
    assert LN_DUE[3] <= KD
    for n in range(S // T0):
        t = n + 1
        if XO[1] <= t < S // T0:
            if t in XO:
                x_copy(XO.index(t)).wait()
                if t == XO[1]:
                    x_copy(3).start()
                if t == XO[2]:
                    kv_start(0, 0)
                    for cp in w_copies(1):
                        cp.start()
                prev = None
            stages = layernorm(t * T0, T0, prev)
            for a in LN_DUE:
                due.setdefault(n * KD + a, []).append(stages)
        if n == S // T0 - 2:
            for cp in w_copies(2):
                cp.start()
        r = pl.ds(n * T0, T0)
        acc = None
        for k in range(KD):
            ks = slice(k * 128, (k + 1) * 128)
            vs = [_rows(jnp.broadcast_to(next(stages), (T0, 128)), 8) for stages in due.pop(n * KD + k, [])]
            deps = {a: [v[2 * a] for v in vs] for a in range(T0 // 16)} if vs else {}
            d = _dot(_after_rows(xn_vm[r, ks], deps, zero0), wq0_vm[ks, :])
            acc = d if acc is None else acc + d
            if k == 3:
                prev = d[:, 0:128]
        for c, qc in enumerate(_cols(acc * QSCALE)):
            q_vm[c, r, :] = qc.astype(bf16)
    assert not due
    for a in range(2):
        rb = _round(router[a])
        rb = jnp.where(rb == 0.0, 0.0, rb)
        bits = lax.shift_right_logical(pltpu.bitcast(rb, i32), 16)
        u = jnp.where(bits >= 0x8000, 0xFFFF - bits, bits + 0x8000)
        u = jnp.where(rb != rb, 0, u)
        key_vm[a] = pltpu.bitcast((1 << 29) + u * S + (S - 1 - (a * 1024 + lane * 8 + sub)), f32)
    for cp in w_copies(1):
        cp.wait()

    def step(g, carry):
        slot = g & 1
        kv_wait(slot)

        @pl.when(g == 1)
        def _():
            for cp in w_copies(2):
                cp.wait()
            row16 = lax.broadcasted_iota(i32, (16, D), 0)
            kbits = pltpu.bitcast(key_vm[2], i32)
            xsel = jnp.zeros((16, D), f32)
            for c in range(C):
                tok = _token(kbits[c, 0])
                grp = xn_vm[_token_group(tok), :].astype(f32)
                rowv = jnp.sum(jnp.where(row16 == (tok & 15), grp, 0.0), axis=0, keepdims=True)
                xsel = jnp.where(row16 == c, rowv, xsel)
            sel_vm[...] = xsel[0:C, :]

        zero = lax.shift_right_logical(g, 8)

        st = dict(k0=key_vm[0], k1=key_vm[1], keys=jnp.zeros((8, 128), f32))
        f0 = pl.multiple_of(jnp.clip((g - 1) * FB, 0, F - FB), 64)

        def pick(c):
            k0, k1 = st["k0"], st["k1"]
            mx = jnp.max(jnp.max(jnp.maximum(k0, k1), axis=1, keepdims=True), axis=0, keepdims=True)
            st["k0"] = jnp.where(k0 == mx, 0.0, k0)
            st["k1"] = jnp.where(k1 == mx, 0.0, k1)
            st["keys"] = jnp.where(sub == c, mx, st["keys"])
            if c == C - 1:
                key_vm[2] = st["keys"]
            return {0: [st["keys"]]}

        def gate_up(k):
            ks = slice(k * 256, min((k + 1) * 256, D))
            w = jnp.concatenate([wf_vm[0, pl.ds(f0, FB), ks], wf_vm[1, pl.ds(f0, FB), ks]], axis=0)
            d = _dot_nt(sel_vm[:, ks].astype(bf16), w)
            st["gu"] = d if k == 0 else st["gu"] + d
            return {}

        def hidden():
            unit_id = f0 + lax.broadcasted_iota(i32, (C, FB), 1)
            gate, up = _cols(st["gu"], FB)
            fresh = unit_id >= jnp.where(g == 0, F, (g - 1) * FB)
            st["hid"] = _round(jnp.where(fresh, gate * _sigmoid(gate) * up, 0.0))
            return {0: [st["hid"]]}

        def down(n):
            cs = slice(n * 512, min((n + 1) * 512, D))
            y_vm[:, cs] += _dot(st["hid"].astype(bf16), wf_vm[2, pl.ds(f0, FB), cs])
            return {}

        tasks = {}
        for c in range(C):
            tasks.setdefault((1 + c // 4 * 2, 0), []).append(lambda c=c: pick(c))
        for k in range(3):
            tasks.setdefault((3, k), []).append(lambda k=k: gate_up(k))
        tasks[4, 0] = [hidden]
        tasks[5, 2] = [lambda: down(0), lambda: down(1)]

        def routed(j, a):
            return ([{}] + [f() for f in tasks.get((j, a), [])])[-1]

        def unit(j):
            u = g * NU + j
            return u >> 3, pl.multiple_of((u & 7) * TQ, TQ)

        def q_unit(j):
            p, r0 = unit(j)
            r = pl.ds(r0, TQ)
            ds = [_dot(_after_rows(xn_vm[r, a * 256:(a + 1) * 256], routed(j, a), zero),
                       wq_vm[p, a * 256:(a + 1) * 256, :]) for a in range(2)]
            q = ds[0] + ds[1]
            rest = [_dot(_after_rows(xn_vm[pl.ds(r0 + a * 128, 128), 512:D], routed(j, 2 + a), zero),
                         wq_vm[p, 512:D, :]) for a in range(2)]
            q = (q + jnp.concatenate(rest, axis=0)) * QSCALE
            for c, qc in enumerate(_cols(q)):
                q_vm[2 * p + 4 + c, r, :] = qc.astype(bf16)
            return ds[1][:, 0:128]

        def o_unit(j):
            p, r0 = unit(j)
            o = jnp.concatenate([o_vm[2 * p + c, pl.ds(r0, TQ), :] for c in range(2)], axis=1)
            left = jnp.concatenate([_dot(o, wo_vm[p, :, a * 256:(a + 1) * 256]) for a in range(2)], axis=1)
            right = jnp.concatenate([_dot(oa, wo_vm[p, :, 512:D]) for oa in _rows(o, 128)], axis=0)
            s_vm[pl.ds(r0, TQ), :] += jnp.concatenate([left, right], axis=1)
            return right

        pending = []

        def store_o(dep):
            t, o = pending.pop()
            deps = {} if dep is None else {a: [d] for a, d in enumerate(_rows(dep, 8)[::2])}
            o_vm[g * 2 + t["h"], t["r"], :] = _after_rows(o, deps, zero)

        def scores(n):
            t = dict(h=n // NR, r=pl.ds(n % NR * TQ, TQ), s=[], sum=None)
            q = q_vm[g * 2 + t["h"], t["r"], :]
            t["unit"] = q_unit(n) if n < NU else None
            for c in range(NC):
                s = _cols(_dot_nt(q, kv_vm[slot, 0, t["h"], c * CK:(c + 1) * CK, :]))
                mc = _fold(s, jnp.maximum)
                m = mc if c == 0 else jnp.maximum(m, mc)
                t["s"].append(s)
                if c == 0 and pending:
                    store_o(s[0])
            t["max"] = jnp.broadcast_to(jnp.max(m, axis=-1, keepdims=True), (TQ, 128))
            return t

        def probs(t, c, dep):
            t["max"] = _after(t["max"], [t["sum"], dep], zero)
            ps = [jnp.exp2(s - t["max"]) for s in t["s"][c]]
            part = _fold(ps, jnp.add)
            t["sum"] = part if c == 0 else t["sum"] + part
            return jnp.concatenate(ps, axis=1).astype(bf16)

        cur = scores(0)
        for n in range(2 * NR):
            if n == 3:
                kv_start(jnp.minimum(g + 1, NP - 1), 1 - slot)
            nxt = scores(n + 1) if n + 1 < 2 * NR else None
            if n == 0:
                last = nxt["unit"]
            for c in range(NC):
                last = _dot(probs(cur, c, last), kv_vm[slot, 1, cur["h"], c * CK:(c + 1) * CK, :])
                acc = last if c == 0 else last + acc
            l = jnp.sum(cur["sum"], axis=-1, keepdims=True)
            rl = pl.reciprocal(l, approx=True)
            last = acc * (rl * (2.0 - l * rl))
            done = o_unit(n - NR - 1) if n > NR else None
            pending.append((cur, last.astype(bf16)))
            if n <= NR or n + 2 >= 2 * NR:
                store_o(done)
            cur = nxt
        assert not pending
        return carry

    lax.fori_loop(0, NP, step, 0)
    kv_wait(NP & 1)

    kbits = pltpu.bitcast(key_vm[2], i32)
    u = lax.shift_right_logical(kbits, 11) & 0xFFFF
    rsel = pltpu.bitcast(jnp.where(u >= 0x8000, u - 0x8000, 0xFFFF - u) << 16, f32)
    bsel = sel_vm[...] + y_vm[...] * jnp.tile(_sigmoid(rsel), (1, KD))
    row16 = lax.broadcasted_iota(i32, (16, D), 0)
    for c in range(C):
        tok = _token(kbits[c, 0])
        grp = xn_vm[_token_group(tok), :].astype(f32)
        xn_vm[_token_group(tok), :] = jnp.where(row16 == (tok & 15), bsel[c:c + 1, :], grp).astype(bf16)

    for n in range(NR):
        r = pl.ds(n * TQ, TQ)
        sent = 0
        for k in range(KD):
            cs = slice(k * 128, (k + 1) * 128)
            b = xn_vm[r, cs].astype(f32)
            gate = b * _sigmoid(b)
            o = jnp.concatenate([o_vm[H - 4 + a, r, :] for a in range(4)], axis=1)
            if n > 0:
                o = _after_rows(o, {a: [d] for a, d in enumerate(_rows(gate, 8)[1::2])}, zero0)
            s = s_vm[r, cs] + _dot(o, jnp.concatenate([wo_vm[NP - 2, :, cs], wo_vm[NP - 1, :, cs]], axis=0))
            out_vm[r, cs] = (x_vm[r, cs].astype(f32) + s * gate).astype(bf16)
            if k == KD - 1 or (n == NR - 1 and k > 0):
                cc = pl.ds(sent * 128, (k + 1 - sent) * 128)
                pltpu.make_async_copy(out_vm.at[r, cc], out_hbm.at[r, cc], io_sem.at[0]).start()
                sent = k + 1
    pltpu.make_async_copy(out_vm, out_hbm, io_sem.at[0]).wait()


@jax.jit
def pallas_recurrent_scan__mha_block_cached__moe_arch_mod__prompt_kernel(
    A_x: jax.Array,
    A_k_cache: jax.Array,
    A_v_cache: jax.Array,
    A_wq: jax.Array,
    A_wo: jax.Array,
    B_x: jax.Array,
    B_w_r: jax.Array,
    B_w_gate: jax.Array,
    B_w_up: jax.Array,
    B_w_down: jax.Array,
):
    del B_x
    hbm = pl.BlockSpec(memory_space=pltpu.HBM)
    dma = pltpu.SemaphoreType.DMA
    out = pl.pallas_call(
        _kernel,
        in_specs=[hbm] * 9,
        out_specs=hbm,
        out_shape=jax.ShapeDtypeStruct((S, D), bf16),
        scratch_shapes=[
            pltpu.VMEM((S, D), bf16),
            pltpu.VMEM((S, D), bf16),
            pltpu.VMEM((H, S, DH), bf16),
            pltpu.VMEM((H, S, DH), bf16),
            pltpu.VMEM((S, D), f32),
            pltpu.VMEM((D, 512), bf16),
            pltpu.VMEM((NP - 2, D, 256), bf16),
            pltpu.VMEM((NP, 256, D), bf16),
            pltpu.VMEM((3, F, D), bf16),
            pltpu.VMEM((2, 2, 2, S, DH), bf16),
            pltpu.VMEM((S, D), bf16),
            pltpu.VMEM((D,), bf16),
            pltpu.VMEM((3, 8, 128), f32),
            pltpu.VMEM((C, D), f32),
            pltpu.VMEM((C, D), f32),
            dma((2,)), dma((2,)), dma((1,)), dma((1,)),
        ],
        compiler_params=pltpu.CompilerParams(vmem_limit_bytes=110 * 2**20),
    )(A_x.reshape(S, D), A_k_cache.reshape(H, S, DH), A_v_cache.reshape(H, S, DH), A_wq,
      A_wo.reshape(NP, 256, D), B_w_r, B_w_gate.T, B_w_up.T, B_w_down)
    return out.reshape(1, S, D)
```
